```python
import os as _os
_os.environ.setdefault("JAX_PLATFORMS", "cpu")
import jax
import jax.numpy as jnp

def _softmax(x, axis=-1):
    return jax.nn.softmax(x, axis=axis)
def _gelu(x):
    return jax.nn.gelu(x, approximate=True)
def _silu(x):
    return jax.nn.silu(x)
def _sigmoid(x):
    return jax.nn.sigmoid(x)
def _layernorm(x, axis=-1, eps=1e-5):
    m = jnp.mean(x, axis=axis, keepdims=True)
    v = jnp.var(x, axis=axis, keepdims=True)
    return (x - m) / jnp.sqrt(v + eps)
def _scatter_add(tgt, idx, src, axis=0):
    return tgt.at[idx].add(src)
def _segment_sum(src, seg, n):
    return jax.ops.segment_sum(src, seg, n)
class _Rng:
    def __init__(self, key):
        self._k = key
    def _next(self):
        self._k, sub = jax.random.split(self._k)
        return sub
    def normal(self, shape):
        return jax.random.normal(self._next(), shape, dtype=jnp.bfloat16)
    def randint(self, lo, hi, shape):
        return jax.random.randint(self._next(), shape, lo, hi, dtype=jnp.int32)
    def uniform(self, shape, lo=0.0, hi=1.0):
        return jax.random.uniform(self._next(), shape, jnp.bfloat16, lo, hi)
    def permutation(self, n):
        return jax.random.permutation(self._next(), n)


kernel_name = 'gated_mix__mha_block__linear_kernel_hedgehog__prompt'

def setup_inputs():
    _rng = _Rng(jax.random.key(int.from_bytes(__import__("os").urandom(4), "little")))
    _w = (lambda a: (lambda t: t.astype(jnp.bfloat16) if jnp.issubdtype(t.dtype, jnp.floating) else t)(jnp.asarray(a)))
    def _A_setup():
        B, S, D, H = 1, 2048, 640, 32
        return {
            "x": _w((lambda *s: _rng.normal(s) * 0.05)(B, S, D)),
            "wqkv": _w((lambda *s: _rng.normal(s) * 0.4)(D, 3 * D)),
            "wo": _w((lambda *s: _rng.normal(s) * 0.05)(D, D)),
        }
    _A_in = _A_setup()

    def _B_setup():
        B, S, D, H = 1, 2048, 640, 32
        Dh = D // H
        return {
            "x": _w((lambda *s: _rng.normal(s) * 0.05)(B, S, D)),
            "wqkv": _w((lambda *s: _rng.normal(s) * 0.8)(D, 3 * D)),
            "w_phi": _w((lambda *s: _rng.normal(s) * 0.8)(H, Dh, Dh) * (Dh ** -0.5)),
            "wo": _w((lambda *s: _rng.normal(s) * 0.05)(D, D)),
        }
    _B_in = _B_setup()

    return {
        "A_x": _A_in["x"],
        "A_wqkv": _A_in["wqkv"],
        "A_wo": _A_in["wo"],
        "B_x": _B_in["x"],
        "B_wqkv": _B_in["wqkv"],
        "B_w_phi": _B_in["w_phi"],
        "B_wo": _B_in["wo"],
        "gate_w": _w((lambda *s: _rng.normal(s) * 0.05)(640) * 16.0),
    }

def reference(A_x, A_wqkv, A_wo, B_x, B_wqkv, B_w_phi, B_wo, gate_w):
    def _A_ref(x, wqkv, wo):
        B, S, D = x.shape
        H = 32
        Dh = D // H
        qkv = (lambda x, *d: x.transpose(*d))((x @ wqkv).reshape(B, S, 3, H, Dh), 2, 0, 3, 1, 4)
        q, k, v = qkv[0], qkv[1], qkv[2]
        scores = jnp.einsum("bhqd,bhkd->bhqk", q, k) * (Dh ** -0.5)
        p = _softmax(scores, axis=-1)
        o = jnp.einsum("bhqk,bhkd->bhqd", p, v)
        return (lambda x, *d: x.transpose(*d))(o, 0, 2, 1, 3).reshape(B, S, D) @ wo

    def _B_ref(x, wqkv, w_phi, wo):
        B, S, D = x.shape
        H = 32; Dh = D // H
        qkv = (lambda x, *d: x.transpose(*d))((x @ wqkv).reshape(B, S, 3, H, Dh), 2, 0, 3, 1, 4)
        q, k, v = qkv[0], qkv[1], qkv[2]
        pq = jnp.einsum("bhsd,hdf->bhsf", q, w_phi)
        pk = jnp.einsum("bhsd,hdf->bhsf", k, w_phi)
        phi_q = jnp.concatenate([_softmax(pq, axis=-1), _softmax(-pq, axis=-1)], axis=-1)
        phi_k = jnp.concatenate([_softmax(pk, axis=-1), _softmax(-pk, axis=-1)], axis=-1)
        kv = jnp.einsum("bhsf,bhsd->bhfd", phi_k, v)
        z  = jnp.einsum("bhsf->bhf", phi_k)
        num = jnp.einsum("bhqf,bhfd->bhqd", phi_q, kv)
        den = jnp.einsum("bhqf,bhf->bhq", phi_q, z)[..., None] + 1e-6
        o = num / den
        return (lambda x, *d: x.transpose(*d))(o, 0, 2, 1, 3).reshape(B, S, D) @ wo

    x = A_x
    g = _sigmoid((x * gate_w).sum(-1, keepdims=True))
    a = _A_ref(x, A_wqkv, A_wo)
    b = _B_ref(x, B_wqkv, B_w_phi, B_wo)
    return g * a + (1 - g) * b
```

```python
import jax
import jax.numpy as jnp
from jax import lax
import jax.experimental.pallas as pl
import jax.experimental.pallas.tpu as pltpu

F32 = jnp.float32
BF16 = jnp.bfloat16
I32 = jnp.int32
U32 = jnp.uint32
I8 = jnp.int8

S = 2048
D = 640
H = 32
DH = 20
NP = H // 2
TS = 512
NTS = S // TS
LOG2E = 1.4426950408889634
QSCALE = (DH ** -0.5) * LOG2E
FS = 1911.0
MAGIC = 12582912.0 + 136.0
TINY = 1e-30
B_MAX = 32.0
V_MIN = 2.0 ** -40

NT_DIMS = (((1,), (1,)), ((), ()))
TN_DIMS = (((0,), (0,)), ((), ()))

TQ = 512
CH = 256
SK = 1


def _dot(a, b):
    return jnp.dot(a, b, preferred_element_type=F32)


def _dot_nt(a, b):
    return lax.dot_general(a, b, NT_DIMS, preferred_element_type=F32)


def _lower(n):
    return lax.broadcasted_iota(I32, (8, n), 0) < 4


def _seg_reduce(v, op, red, fill, low):
    a = op(op(v[0], v[1]), jnp.where(low, v[2], fill))
    b = op(op(v[3], v[4]), jnp.where(low, fill, v[2]))
    return red(a, axis=0, keepdims=True), red(b, axis=0, keepdims=True)


def _seg_bcast(a, b, low):
    n = a.shape[-1]
    a8 = jnp.broadcast_to(a, (8, n))
    b8 = jnp.broadcast_to(b, (8, n))
    return [a8, a8, jnp.where(low, a8, b8), b8, b8]


def _tiles(z):
    return [z[8 * i:8 * (i + 1)] for i in range(z.shape[0] // 8)]


def _feature_softmax(z):
    n = z.shape[-1]
    low = _lower(n)
    v = _tiles(z)
    mx = _seg_bcast(*_seg_reduce(v, jnp.maximum, jnp.max, -jnp.inf, low), low)
    mn = _seg_bcast(*_seg_reduce(v, jnp.minimum, jnp.min, jnp.inf, low), low)
    ep = [jnp.exp2(a - m) for a, m in zip(v, mx)]
    en = [jnp.exp2(m - a) for a, m in zip(v, mn)]
    sa, sb = _seg_reduce(ep, jnp.add, jnp.sum, 0.0, low)
    rp = _seg_bcast(1.0 / sa, 1.0 / sb, low)
    sa, sb = _seg_reduce(en, jnp.add, jnp.sum, 0.0, low)
    rn = _seg_bcast(1.0 / sa, 1.0 / sb, low)
    return jnp.concatenate([e * r for e, r in zip(ep, rp)] + [e * r for e, r in zip(en, rn)], axis=0)


def _head_blocks(slots, low):
    zero = jnp.zeros_like(slots[0][0])
    blk_a, blk_b = [], []
    for t in range(6):
        blk_a += [slots[t][0], slots[t][1]]
        blk_b += [slots[t][3], slots[t][4]]
    for t in range(0, 6, 2):
        lo, hi = slots[t][2], slots[t + 1][2]
        blk_a.append(jnp.where(low, lo, pltpu.roll(hi, 4, 0)))
        blk_b.append(jnp.where(low, pltpu.roll(lo, 4, 0), hi))
    blk_a.append(zero)
    blk_b.append(zero)
    return jnp.concatenate(blk_a, axis=0), jnp.concatenate(blk_b, axis=0)


def _kernel(x_hbm, wa_hbm, woa_hbm, wb_hbm, wphi_hbm, wob_hbm, gate_hbm, out_hbm,
            x_v, wa_v, wb_v, wo_v, wphi_v, gate_v, wt1, wt2, xs, kt, kcol, kv, lmat,
            q8t, k8, vt, sc, g_v, ot, ostage, chk, qtf, in_sems, out_sems):
    copies = [
        pltpu.make_async_copy(x_hbm.at[0], x_v, in_sems.at[0]),
        pltpu.make_async_copy(wa_hbm, wa_v, in_sems.at[1]),
        pltpu.make_async_copy(wb_hbm, wb_v, in_sems.at[2]),
        pltpu.make_async_copy(wphi_hbm, wphi_v, in_sems.at[3]),
        pltpu.make_async_copy(gate_hbm, gate_v, in_sems.at[4]),
        pltpu.make_async_copy(woa_hbm, wo_v.at[0:D], in_sems.at[5]),
        pltpu.make_async_copy(wob_hbm, wo_v.at[D:2 * D], in_sems.at[6]),
    ]
    for c in copies:
        c.start()

    copies[1].wait()
    wt1[0:D, :] = wa_v[:, D:2 * D].T
    wt2[D:2 * D, :] = wa_v[:, 0:D].T
    wt2[2 * D:3 * D, :] = wa_v[:, 2 * D:3 * D].T
    copies[2].wait()
    copies[3].wait()
    copies[4].wait()
    wt1[2 * D:3 * D, :] = wb_v[:, 2 * D:3 * D].T
    w2 = wphi_v[...].astype(F32).reshape(D, DH)
    w2t = jnp.concatenate([w2, jnp.zeros((D, 128 - DH), F32)], axis=1).T
    er = lax.broadcasted_iota(I32, (D, 128), 0) % DH
    ec = lax.broadcasted_iota(I32, (D, 128), 1)
    rep = _dot((er == ec).astype(BF16), w2t.astype(BF16))
    br = lax.broadcasted_iota(I32, (D, D), 0) // DH
    bc = lax.broadcasted_iota(I32, (D, D), 1) // DH
    bdt = jnp.where(br == bc, rep, 0.0).astype(BF16)
    wt1[D:2 * D, :] = (_dot_nt(bdt, wb_v[:, D:2 * D]) * LOG2E).astype(BF16)
    wt2[0:D, :] = (_dot_nt(bdt, wb_v[:, 0:D]) * LOG2E).astype(BF16)
    grow = jnp.broadcast_to(gate_v[...].astype(F32).reshape(1, D), (16, D))
    wt2[3 * D:3 * D + 16, :] = grow.astype(BF16)

    kcol[...] = jnp.zeros_like(kcol)
    kv[...] = jnp.zeros_like(kv)
    chk[...] = jnp.concatenate([jnp.ones((8, 128), F32), jnp.zeros((8, 128), F32)], axis=0)
    copies[0].wait()

    def phase1(j, carry):
        r0 = pl.multiple_of(j * TS, TS)
        for c in range(5):
            xs[c] = x_v[pl.ds(r0, TS), 128 * c:128 * (c + 1)].astype(F32)
        xp = jnp.concatenate(
            [jnp.concatenate([xs[c, pl.ds(b, 128, stride=4), :] for c in range(5)], axis=1)
             for b in range(4)], axis=0).astype(BF16)
        k_t = _dot_nt(wt1[0:D, :], xp)
        kt[:, pl.ds(r0, TS)] = k_t
        ak = jnp.abs(k_t)
        m = ak[:, 0:128]
        fin = ak[:, 0:128] < jnp.inf
        for b in range(1, 4):
            m = jnp.maximum(m, ak[:, 128 * b:128 * (b + 1)])
            fin = jnp.logical_and(fin, ak[:, 128 * b:128 * (b + 1)] < jnp.inf)
        kcol[...] = jnp.maximum(kcol[...], m)
        okf = jnp.min(jnp.where(fin, 1.0, 0.0).reshape(D // 8, 8, 128), axis=0)
        chk[0:8, :] = jnp.minimum(chk[0:8, :], okf)
        pk_t = _dot_nt(wt1[D:2 * D, :], xp)
        vb_t = _dot_nt(wt1[2 * D:3 * D, :], xp)
        ones8 = jnp.where(lax.broadcasted_iota(I32, (8, TS), 0) == 0, 1.0, 0.0)
        for p in range(NP):
            phi = _feature_softmax(pk_t[40 * p:40 * (p + 1)]).astype(BF16)
            vaug = jnp.concatenate([vb_t[40 * p:40 * (p + 1)], ones8], axis=0).astype(BF16)
            kv[p, :, 0:80] = kv[p, :, 0:80] + _dot_nt(vaug, phi)
        return carry

    lax.fori_loop(0, NTS, phase1, 0)

    kc = jnp.maximum(jnp.max(kcol[...], axis=1, keepdims=True), TINY)
    kcol[...] = jnp.broadcast_to(kc, (D, 128))
    kvv = kv[...]
    r = lax.broadcasted_iota(I32, (NP, 48, 128), 1)
    c = lax.broadcasted_iota(I32, (NP, 48, 128), 2)
    col_a = (c < 20) | ((c >= 40) & (c < 60))
    col_b = ((c >= 20) & (c < 40)) | ((c >= 60) & (c < 80))
    row_a = (r < 20) | (r == 40)
    row_b = ((r >= 20) & (r < 40)) | (r == 41)
    src = jnp.where(r >= 40, jnp.broadcast_to(kvv[:, 40:41, :], (NP, 48, 128)), kvv)
    lmat[...] = jnp.where((row_a & col_a) | (row_b & col_b), src, 0.0).astype(BF16)

    def phase2(j, carry):
        r0 = pl.multiple_of(j * TS, TS)
        cols = pl.ds(r0, TS)
        xt = x_v[cols, :]
        g = jax.nn.sigmoid(_dot_nt(wt2[3 * D:3 * D + 16, :], xt)[0:1])
        g_v[:, cols] = jnp.broadcast_to(g, (8, TS))
        low = _lower(TS)
        pq_t = _dot_nt(wt2[0:D, :], xt)
        for p in range(NP):
            phi = _feature_softmax(pq_t[40 * p:40 * (p + 1)]).astype(BF16)
            nd = _dot(lmat[p, :, 0:80], phi)
            rr = _seg_bcast((1.0 - g) / (nd[40:41] + 1e-6), (1.0 - g) / (nd[41:42] + 1e-6), low)
            ob = jnp.concatenate([a * b for a, b in zip(_tiles(nd[0:40]), rr)], axis=0)
            ot[D + 40 * p:D + 40 * (p + 1), cols] = ob.astype(BF16)
        va_t = _dot_nt(wt2[2 * D:3 * D, :], xt)
        sub = lax.broadcasted_iota(I32, (8, TS), 0)
        zero8 = jnp.zeros((8, TS), F32)
        vm = jnp.zeros((8, 128), F32)
        av = jnp.max(jnp.abs(va_t).reshape(D // 8, 8, TS), axis=0)
        for b in range(4):
            vm = jnp.maximum(vm, av[:, 128 * b:128 * (b + 1)])
        chk[8:16, :] = jnp.maximum(chk[8:16, :], vm)
        for p in range(NP):
            v = _tiles(va_t[40 * p:40 * (p + 1)])
            mid_a = jnp.where(low, v[2], jnp.where(sub == 4, 1.0, 0.0))
            mid_b = jnp.where(low, jnp.where(sub == 0, 1.0, 0.0), v[2])
            vt[2 * p, :, cols] = jnp.concatenate([v[0], v[1], mid_a, zero8], axis=0).astype(BF16)
            vt[2 * p + 1, :, cols] = jnp.concatenate([v[3], v[4], mid_b, zero8], axis=0).astype(BF16)
        q_t = _dot_nt(wt2[D:2 * D, :], xt)
        low1 = _lower(128)
        ok = jnp.ones((1, 128), F32)
        for p in range(NP):
            kcp = kcol[40 * p:40 * (p + 1), :] * QSCALE
            for t in range(4):
                tc = pl.ds(r0 + 128 * t, 128)
                z = _tiles(q_t[40 * p:40 * (p + 1), 128 * t:128 * (t + 1)] * kcp)
                az = [jnp.abs(a) for a in z]
                bnd_a, bnd_b = _seg_reduce(az, jnp.add, jnp.sum, 0.0, low1)
                m_a, m_b = _seg_reduce(az, jnp.maximum, jnp.max, 0.0, low1)
                m_a = jnp.maximum(m_a, TINY)
                m_b = jnp.maximum(m_b, TINY)
                inv = _seg_bcast(FS / m_a, FS / m_b, low1)
                bits = [lax.bitcast_convert_type(a * i + MAGIC, I32) for a, i in zip(z, inv)]
                x0 = [(u << 20) >> 28 for u in bits]
                x1 = [((u >> 4) & 15) - 8 for u in bits]
                x2 = [(u & 15) - 8 for u in bits]
                slots = [[a << 4 for a in x0], [a << 2 for a in x0], [a << 2 for a in x1], x1, x0, x2]
                blk_a, blk_b = _head_blocks(slots, low1)
                q8t[2 * p, :, tc] = blk_a.astype(I8)
                q8t[2 * p + 1, :, tc] = blk_b.astype(I8)
                z6 = jnp.zeros((6, 128), F32)
                sc[2 * p, :, tc] = jnp.concatenate([m_a * (256.0 / (FS * FS)), -bnd_a, z6], axis=0)
                sc[2 * p + 1, :, tc] = jnp.concatenate([m_b * (256.0 / (FS * FS)), -bnd_b, z6], axis=0)
                ok = jnp.minimum(ok, jnp.where(jnp.logical_and(bnd_a <= B_MAX, bnd_b <= B_MAX), 1.0, 0.0))
        chk[0:1, :] = jnp.minimum(chk[0:1, :], ok)
        for p in range(NP):
            kinv = FS / kcol[40 * p:40 * (p + 1), :]
            w0 = w1 = w2_ = None
            for b in range(4):
                y = kt[40 * p:40 * (p + 1), pl.ds(r0 + 128 * b, 128)] * kinv + MAGIC
                u = lax.bitcast_convert_type(y, U32)
                msk = jnp.uint32(15 << (8 * b))
                n2 = (u << (8 * b)) & msk
                n1 = ((u >> 4) if b == 0 else (u << (8 * b - 4))) & msk
                n0 = ((u >> 8) if b == 0 else (u if b == 1 else (u << (8 * b - 8)))) & msk
                w0 = n0 if b == 0 else w0 | n0
                w1 = n1 if b == 0 else w1 | n1
                w2_ = n2 if b == 0 else w2_ | n2
            c78 = jnp.uint32(0x78787878)
            c80 = jnp.uint32(0x80808080)
            w0 = ((w0 ^ jnp.uint32(0x08080808)) + c78) ^ c80
            w1 = (w1 + c78) ^ c80
            w2_ = (w2_ + c78) ^ c80
            cf0 = jnp.uint32(0xF0F0F0F0)
            cfc = jnp.uint32(0xFCFCFCFC)
            slots = [_tiles((w0 << 4) & cf0), _tiles((w1 << 2) & cfc), _tiles((w0 << 2) & cfc),
                     _tiles(w1), _tiles(w2_), _tiles(w0)]
            blk_a, blk_b = _head_blocks(slots, low1)
            k8[2 * p, cols, :] = pltpu.bitcast(lax.bitcast_convert_type(blk_a, I32).T, I8)
            k8[2 * p + 1, cols, :] = pltpu.bitcast(lax.bitcast_convert_type(blk_b, I32).T, I8)
        return carry

    lax.fori_loop(0, NTS, phase2, 0)

    fast = jnp.logical_and(jnp.min(chk[0:8, :]) > 0.5, jnp.max(chk[8:16, :]) >= V_MIN)

    def finish_pair(p, acc_a, acc_b, cols, n):
        low = _lower(n)
        g = g_v[0:1, cols]
        ra = g / acc_a[20:21]
        rb = g / acc_b[16:17]
        o = jnp.concatenate([acc_a[0:8] * ra, acc_a[8:16] * ra,
                             jnp.where(low, acc_a[16:24] * ra, acc_b[16:24] * rb),
                             acc_b[0:8] * rb, acc_b[8:16] * rb], axis=0)
        ot[pl.ds(pl.multiple_of(40 * p, 8), 40), cols] = o.astype(BF16)

    @pl.when(fast)
    def _():
        nq = S // TQ
        nt = TQ // 128
        nch = S // CH

        def pair_body(p, carry):
            steps = [(qi, u) for qi in range(nq) for u in range(2)]
            pv = {}
            acc = {}

            def stage_a(g):
                s, j = divmod(g, nch)
                qi, u = steps[s]
                h = 2 * p + u
                z = jnp.dot(k8[h, j * CH:(j + 1) * CH, :], q8t[h, :, qi * TQ:(qi + 1) * TQ],
                            preferred_element_type=I32)
                for t in range(nt):
                    c0 = qi * TQ + t * 128
                    sig = sc[h, 0:1, c0:c0 + 128]
                    nb = sc[h, 1:2, c0:c0 + 128]
                    pv[(g, t)] = jnp.exp2(z[:, t * 128:(t + 1) * 128].astype(F32) * sig + nb)

            def stage_b(g):
                s, j = divmod(g, nch)
                qi, u = steps[s]
                h = 2 * p + u
                v = vt[h, :, j * CH:(j + 1) * CH]
                ds = [_dot(v, pv.pop((g, t)).astype(BF16))[0:24] for t in range(nt)]
                acc[s] = ds if j == 0 else [a + b for a, b in zip(acc[s], ds)]
                if j == nch - 1 and u == 1:
                    for t in range(nt):
                        c0 = qi * TQ + t * 128
                        finish_pair(p, acc[s - 1][t], acc[s][t], pl.ds(c0, 128), 128)

            total = len(steps) * nch
            for g in range(total + SK):
                if g < total:
                    stage_a(g)
                if g >= SK:
                    stage_b(g - SK)
            return carry

        lax.fori_loop(0, NP, pair_body, 0)

    @pl.when(jnp.logical_not(fast))
    def _():
        def proj(j, carry):
            cols = pl.ds(pl.multiple_of(j * TS, TS), TS)
            xt = x_v[cols, :]
            kt[:, cols] = _dot_nt(wt1[0:D, :], xt)
            qtf[:, cols] = _dot_nt(wt2[D:2 * D, :], xt) * QSCALE
            return carry

        lax.fori_loop(0, NTS, proj, 0)
        tf = 256

        def body(i, carry):
            p = i // (S // tf)
            cols = pl.ds(pl.multiple_of((i % (S // tf)) * tf, tf), tf)
            rows = pl.ds(pl.multiple_of(40 * p, 8), 40)
            kp = kt[rows, :].astype(BF16)
            qp = qtf[rows, cols]
            first = lax.broadcasted_iota(I32, (40, tf), 0) < 20
            accs = []
            for u in range(2):
                qm = jnp.where(first if u == 0 else jnp.logical_not(first), qp, 0.0).astype(BF16)
                s_t = lax.dot_general(kp, qm, TN_DIMS, preferred_element_type=F32)
                pr = jnp.exp2(s_t - jnp.max(s_t, axis=0, keepdims=True)).astype(BF16)
                accs.append(_dot(vt[2 * p + u], pr)[0:24])
            finish_pair(p, accs[0], accs[1], cols, tf)
            return carry

        lax.fori_loop(0, NP * (S // tf), body, 0)

    copies[5].wait()
    copies[6].wait()

    def out_copy(j):
        return pltpu.make_async_copy(ostage.at[j % 2], out_hbm.at[0, pl.ds(j * TS, TS), :],
                                     out_sems.at[j % 2])

    for j in range(NTS):
        o = lax.dot_general(ot[:, j * TS:(j + 1) * TS], wo_v[...], TN_DIMS, preferred_element_type=F32)
        if j >= 2:
            out_copy(j - 2).wait()
        ostage[j % 2] = o.astype(BF16)
        out_copy(j).start()
    out_copy(NTS - 2).wait()
    out_copy(NTS - 1).wait()


def _build():
    any_spec = pl.BlockSpec(memory_space=pl.ANY)
    scratch = [
        pltpu.VMEM((S, D), BF16),
        pltpu.VMEM((D, 3 * D), BF16),
        pltpu.VMEM((D, 3 * D), BF16),
        pltpu.VMEM((2 * D, D), BF16),
        pltpu.VMEM((H, DH, DH), BF16),
        pltpu.VMEM((D,), BF16),
        pltpu.VMEM((3 * D, D), BF16),
        pltpu.VMEM((3 * D + 16, D), BF16),
        pltpu.VMEM((5, TS, 128), F32),
        pltpu.VMEM((D, S), F32),
        pltpu.VMEM((D, 128), F32),
        pltpu.VMEM((NP, 48, 128), F32),
        pltpu.VMEM((NP, 48, 128), BF16),
        pltpu.VMEM((H, 128, S), I8),
        pltpu.VMEM((H, S, 128), I8),
        pltpu.VMEM((H, 32, S), BF16),
        pltpu.VMEM((H, 8, S), F32),
        pltpu.VMEM((8, S), F32),
        pltpu.VMEM((2 * D, S), BF16),
        pltpu.VMEM((2, TS, D), BF16),
        pltpu.VMEM((16, 128), F32),
        pltpu.VMEM((D, S), F32),
        pltpu.SemaphoreType.DMA((7,)),
        pltpu.SemaphoreType.DMA((2,)),
    ]
    return pl.pallas_call(
        _kernel,
        out_shape=jax.ShapeDtypeStruct((1, S, D), BF16),
        in_specs=[any_spec] * 7,
        out_specs=any_spec,
        scratch_shapes=scratch,
        compiler_params=pltpu.CompilerParams(vmem_limit_bytes=100 * 1024 * 1024),
        name="gated_mix_attn",
    )


@jax.jit
def pallas_gated_mix__mha_block__linear_kernel_hedgehog__prompt_kernel(
    A_x: jax.Array,
    A_wqkv: jax.Array,
    A_wo: jax.Array,
    B_x: jax.Array,
    B_wqkv: jax.Array,
    B_w_phi: jax.Array,
    B_wo: jax.Array,
    gate_w: jax.Array,
):
    del B_x
    return _build()(A_x, A_wqkv, A_wo, B_wqkv, B_w_phi, B_wo, gate_w)
```

```python
import jax
import jax.numpy as jnp
from jax import lax
import jax.experimental.pallas as pl
import jax.experimental.pallas.tpu as pltpu

F32 = jnp.float32
BF16 = jnp.bfloat16
I32 = jnp.int32
U32 = jnp.uint32
I8 = jnp.int8

S = 2048
D = 640
H = 32
DH = 20
NP = H // 2
TS = 512
NTS = S // TS
GP = 16
GR = 40 * GP
NG = NP // GP
LOG2E = 1.4426950408889634
QSCALE = (DH ** -0.5) * LOG2E
FS = 1911.0
MAGIC = 12582912.0 + 136.0
TINY = 1e-30
Q_MAX = 3.0
V_MIN = 2.0 ** -20
V_MAX = 2.0 ** 60

NT_DIMS = (((1,), (1,)), ((), ()))
TN_DIMS = (((0,), (0,)), ((), ()))

TQ = 512
CH = 256
CB = 128
SK = 2


def _dot(a, b):
    return jnp.dot(a, b, preferred_element_type=F32)


def _dot_nt(a, b):
    return lax.dot_general(a, b, NT_DIMS, preferred_element_type=F32)


def _recip(x):
    r = pl.reciprocal(x, approx=True)
    return r * (2.0 - x * r)


def _lower(n):
    return lax.broadcasted_iota(I32, (8, n), 0) < 4


def _seg_reduce(v, op, red, fill, low):
    a = op(op(v[0], v[1]), jnp.where(low, v[2], fill))
    b = op(op(v[3], v[4]), jnp.where(low, fill, v[2]))
    return red(a, axis=0, keepdims=True), red(b, axis=0, keepdims=True)


def _seg_bcast(a, b, low):
    n = a.shape[-1]
    a8 = jnp.broadcast_to(a, (8, n))
    b8 = jnp.broadcast_to(b, (8, n))
    return [a8, a8, jnp.where(low, a8, b8), b8, b8]


def _tiles(z):
    return [z[8 * i:8 * (i + 1)] for i in range(z.shape[0] // 8)]


def _feature_softmax(z):
    n = z.shape[-1]
    low = _lower(n)
    v = _tiles(z)
    mx = _seg_bcast(*_seg_reduce(v, jnp.maximum, jnp.max, -jnp.inf, low), low)
    mn = _seg_bcast(*_seg_reduce(v, jnp.minimum, jnp.min, jnp.inf, low), low)
    ep = [jnp.exp2(a - m) for a, m in zip(v, mx)]
    en = [jnp.exp2(m - a) for a, m in zip(v, mn)]
    sa, sb = _seg_reduce(ep, jnp.add, jnp.sum, 0.0, low)
    rp = _seg_bcast(_recip(sa), _recip(sb), low)
    sa, sb = _seg_reduce(en, jnp.add, jnp.sum, 0.0, low)
    rn = _seg_bcast(_recip(sa), _recip(sb), low)
    return jnp.concatenate([e * r for e, r in zip(ep, rp)] + [e * r for e, r in zip(en, rn)], axis=0)


def _head_blocks(slots, low, last_a, last_b):
    blk_a, blk_b = [], []
    for t in range(6):
        blk_a += [slots[t][0], slots[t][1]]
        blk_b += [slots[t][3], slots[t][4]]
    for t in range(0, 6, 2):
        lo, hi = slots[t][2], slots[t + 1][2]
        blk_a.append(jnp.where(low, lo, pltpu.roll(hi, 4, 0)))
        blk_b.append(jnp.where(low, pltpu.roll(lo, 4, 0), hi))
    blk_a.append(last_a)
    blk_b.append(last_b)
    return jnp.concatenate(blk_a, axis=0), jnp.concatenate(blk_b, axis=0)


def _kernel(x_hbm, wa_hbm, woa_hbm, wb_hbm, wphi_hbm, wob_hbm, gate_hbm, out_hbm,
            x_v, xp_v, wak_v, waqv_v, wb_v, wo_v, wot, wphi_v, w2s, gate_v, wt1, wt2, xs, kt, kcol, kinv_v, kv, lmat,
            q8t, k8, vt, sc, g_v, ot, ostage, chk, qtf, in_sems, out_sems):
    cp_x = [pltpu.make_async_copy(x_hbm.at[0, pl.ds(j * TS, TS), :], x_v.at[pl.ds(j * TS, TS), :], in_sems.at[j])
            for j in range(NTS)]
    cp_wk = pltpu.make_async_copy(wa_hbm.at[:, pl.ds(D, D)], wak_v, in_sems.at[4])
    cp_wb = pltpu.make_async_copy(wb_hbm, wb_v, in_sems.at[5])
    cp_phi = pltpu.make_async_copy(wphi_hbm, wphi_v, in_sems.at[6])
    cp_gate = pltpu.make_async_copy(gate_hbm, gate_v, in_sems.at[7])
    cp_wq = pltpu.make_async_copy(wa_hbm.at[:, pl.ds(0, D)], waqv_v.at[:, pl.ds(0, D)], in_sems.at[8])
    cp_wv = pltpu.make_async_copy(wa_hbm.at[:, pl.ds(2 * D, D)], waqv_v.at[:, pl.ds(D, D)], in_sems.at[9])
    cp_woa = pltpu.make_async_copy(woa_hbm, wo_v.at[0:D], in_sems.at[10])
    cp_wob = pltpu.make_async_copy(wob_hbm, wo_v.at[D:2 * D], in_sems.at[11])
    for c in (cp_x[0], cp_wk, cp_x[1], cp_x[2], cp_x[3], cp_wb, cp_phi, cp_gate):
        c.start()
    kcol[...] = jnp.zeros_like(kcol)
    kv[...] = jnp.zeros_like(kv)
    chk[...] = jnp.concatenate([jnp.ones((8, 128), F32), jnp.zeros((8, 128), F32)], axis=0)

    def permute(j):
        r0 = j * TS
        for c in range(5):
            xs[c] = x_v[r0:r0 + TS, 128 * c:128 * (c + 1)].astype(F32)
        for b in range(4):
            xp_v[r0 + 128 * b:r0 + 128 * (b + 1), :] = jnp.concatenate(
                [xs[c, pl.ds(b, 128, stride=4), :] for c in range(5)], axis=1).astype(BF16)

    def keys(j):
        r0 = j * TS
        k_t = _dot_nt(wt1[0:D, :], xp_v[r0:r0 + TS, :])
        kt[:, r0:r0 + TS] = k_t
        ak = jnp.abs(k_t)
        m = ak[:, 0:128]
        fin = ak[:, 0:128] < jnp.inf
        for b in range(1, 4):
            m = jnp.maximum(m, ak[:, 128 * b:128 * (b + 1)])
            fin = jnp.logical_and(fin, ak[:, 128 * b:128 * (b + 1)] < jnp.inf)
        kcol[...] = jnp.maximum(kcol[...], m)
        okf = jnp.min(jnp.where(fin, 1.0, 0.0).reshape(D // 8, 8, 128), axis=0)
        chk[0:8, :] = jnp.minimum(chk[0:8, :], okf)

    cp_x[0].wait()
    permute(0)
    cp_wk.wait()
    cp_x[1].wait()
    wt1[0:D, :] = wak_v[...].T
    permute(1)
    keys(0)
    cp_x[2].wait()
    cp_x[3].wait()
    cp_wv.start()
    cp_wq.start()
    permute(2)
    keys(1)
    permute(3)
    keys(2)
    cp_wb.wait()
    cp_phi.wait()
    cp_gate.wait()
    cp_wv.wait()
    wt2[2 * D + 16:3 * D + 16, :] = waqv_v[:, D:2 * D].T
    wt1[2 * D:3 * D, :] = wb_v[:, 2 * D:3 * D].T
    for blk in range(5):
        rows = []
        for dl in range(4):
            a = wphi_v[4 * blk + dl].astype(F32)
            rows += [jnp.concatenate([a, jnp.zeros((DH, 128 - H), F32)], axis=1), jnp.zeros((12, 128), F32)]
        t = jnp.concatenate(rows, axis=0).T[0:H]
        for dl in range(4):
            w2s[pl.ds(4 * blk + dl, H, stride=DH), :] = t if dl == 0 else pltpu.roll(t, 128 - 32 * dl, 1)
    w2t = w2s[...].T.astype(BF16)
    for i, (k0, k1) in enumerate(((0, 2), (0, 3), (1, 4), (2, 5), (3, 5))):
        rows = lax.broadcasted_iota(I32, (128, 128), 0) + 128 * i
        sel = (rows % DH == lax.broadcasted_iota(I32, (128, 128), 1)).astype(BF16)
        rep = _dot(sel, w2t[:, 128 * k0:128 * k1])
        rh = rows // DH
        blk = []
        for k in range(k0, k1):
            ch = (lax.broadcasted_iota(I32, (8, 128), 1) + 128 * k) // DH
            blk.append(jnp.where(rh == ch[0:1], rep[:, 128 * (k - k0):128 * (k - k0 + 1)], 0.0))
        bdt = jnp.concatenate(blk, axis=1).astype(BF16)
        wt1[D + 128 * i:D + 128 * (i + 1), :] = (
            _dot_nt(bdt, wb_v[:, D + 128 * k0:D + 128 * k1]) * LOG2E).astype(BF16)
        wt2[D + 16 + 128 * i:D + 16 + 128 * (i + 1), :] = (
            _dot_nt(bdt, wb_v[:, 128 * k0:128 * k1]) * LOG2E).astype(BF16)
    grow = jnp.broadcast_to(gate_v[...].astype(F32).reshape(1, D), (16, D))
    wt2[D:D + 16, :] = grow.astype(BF16)
    keys(3)
    kc = jnp.maximum(jnp.max(kcol[...], axis=1, keepdims=True), TINY)
    kinv_v[...] = jnp.broadcast_to(FS / kc, (D, 128))
    kcol[...] = jnp.broadcast_to(kc * QSCALE, (D, 128))
    cp_woa.start()
    cp_wob.start()
    cp_wq.wait()

    def key_digits(p, r0, cols, low1):
        kinv = kinv_v[40 * p:40 * (p + 1), :]
        w0 = w1 = w2_ = None
        for b in range(4):
            y = kt[40 * p:40 * (p + 1), pl.ds(r0 + 128 * b, 128)] * kinv + MAGIC
            u = lax.bitcast_convert_type(y, U32)
            msk = jnp.uint32(15 << (8 * b))
            n2 = (u << (8 * b)) & msk
            n1 = ((u >> 4) if b == 0 else (u << (8 * b - 4))) & msk
            n0 = ((u >> 8) if b == 0 else (u if b == 1 else (u << (8 * b - 8)))) & msk
            w0 = n0 if b == 0 else w0 | n0
            w1 = n1 if b == 0 else w1 | n1
            w2_ = n2 if b == 0 else w2_ | n2
        c78 = jnp.uint32(0x78787878)
        c80 = jnp.uint32(0x80808080)
        w0 = ((w0 ^ jnp.uint32(0x08080808)) + c78) ^ c80
        w1 = (w1 + c78) ^ c80
        w2_ = (w2_ + c78) ^ c80
        cf0 = jnp.uint32(0xF0F0F0F0)
        cfc = jnp.uint32(0xFCFCFCFC)
        slots = [_tiles((w0 << 4) & cf0), _tiles((w1 << 2) & cfc), _tiles((w0 << 2) & cfc),
                 _tiles(w1), _tiles(w2_), _tiles(w0)]
        shift_w = jnp.where(lax.broadcasted_iota(I32, (8, 128), 0) == 0,
                            jnp.uint32(0xFFFFFFFF), jnp.uint32(0x80808080))
        blk_a, blk_b = _head_blocks(slots, low1, shift_w, shift_w)
        k8[2 * p, cols, :] = pltpu.bitcast(lax.bitcast_convert_type(blk_a, I32).T, I8)
        k8[2 * p + 1, cols, :] = pltpu.bitcast(lax.bitcast_convert_type(blk_b, I32).T, I8)

    def phase1(j, carry):
        r0 = pl.multiple_of(j * TS, TS)
        cols = pl.ds(r0, TS)
        xt = x_v[cols, :]
        ones8 = jnp.where(lax.broadcasted_iota(I32, (8, TS), 0) == 0, 1.0, 0.0)
        low1 = _lower(128)
        low = _lower(TS)
        sub = lax.broadcasted_iota(I32, (8, TS), 0)
        zero8 = jnp.zeros((8, TS), F32)
        proj = {}
        state = {"vm": jnp.zeros((8, TS), F32)}

        def mxu(g):
            lo, hi = GR * g, GR * (g + 1)
            proj[g] = (_dot_nt(wt1[D + lo:D + hi, :], xt), _dot_nt(wt1[2 * D + lo:2 * D + hi, :], xt),
                       _dot_nt(wt2[2 * D + 16 + lo:2 * D + 16 + hi, :], xt))

        def vpu(g):
            pk_t, vb_t, va_t = proj.pop(g)
            for i in range(GP):
                p = GP * g + i
                v = _tiles(va_t[40 * i:40 * (i + 1)])
                for a in v:
                    state["vm"] = jnp.maximum(state["vm"], jnp.abs(a))
                mid_a = jnp.where(low, v[2], jnp.where(sub == 4, 1.0, 0.0))
                mid_b = jnp.where(low, jnp.where(sub == 0, 1.0, 0.0), v[2])
                vt[2 * p, :, cols] = jnp.concatenate([v[0], v[1], mid_a, zero8], axis=0).astype(BF16)
                vt[2 * p + 1, :, cols] = jnp.concatenate([v[3], v[4], mid_b, zero8], axis=0).astype(BF16)
                phi = _feature_softmax(pk_t[40 * i:40 * (i + 1)]).astype(BF16)
                vaug = jnp.concatenate([vb_t[40 * i:40 * (i + 1)], ones8], axis=0).astype(BF16)
                kv[p, :, 0:80] = kv[p, :, 0:80] + _dot_nt(vaug, phi)
                key_digits(p, r0, cols, low1)

        for i in range(2):
            r = pl.multiple_of(jnp.minimum(2 * j + i, 4) * 128, 128)
            wt2[pl.ds(r, 128), :] = waqv_v[:, pl.ds(r, 128)].T
        mxu(0)
        for g in range(NG):
            if g + 1 < NG:
                mxu(g + 1)
            vpu(g)
        vm = state["vm"]
        for b in range(4):
            chk[8:16, :] = jnp.maximum(chk[8:16, :], vm[:, 128 * b:128 * (b + 1)])
        return carry

    lax.fori_loop(0, NTS, phase1, 0)

    kvv = kv[...]
    r = lax.broadcasted_iota(I32, (NP, 48, 128), 1)
    c = lax.broadcasted_iota(I32, (NP, 48, 128), 2)
    col_a = (c < 20) | ((c >= 40) & (c < 60))
    col_b = ((c >= 20) & (c < 40)) | ((c >= 60) & (c < 80))
    row_a = (r < 20) | (r == 40)
    row_b = ((r >= 20) & (r < 40)) | (r == 41)
    src = jnp.where(r >= 40, jnp.broadcast_to(kvv[:, 40:41, :], (NP, 48, 128)), kvv)
    lmat[...] = jnp.where((row_a & col_a) | (row_b & col_b), src, 0.0).astype(BF16)

    cp_woa.wait()
    cp_wob.wait()

    def phase2(j, carry):
        r0 = pl.multiple_of(j * TS, TS)
        cols = pl.ds(r0, TS)
        xt = x_v[cols, :]
        for i in range(3):
            r = pl.multiple_of(jnp.minimum(3 * j + i, 9) * 128, 128)
            wot[:, pl.ds(r, 128)] = wo_v[pl.ds(r, 128), :].T
        first = _dot_nt(wt2[0:D + 16, :], xt)
        g = jax.nn.sigmoid(first[D:D + 1])
        g_v[:, cols] = jnp.broadcast_to(g, (8, TS))
        low = _lower(TS)
        low1 = _lower(128)
        shift_q = jnp.full((8, 128), 127, I32)
        proj = {}
        state = {"ok": jnp.ones((1, 128), F32)}

        def mxu(gi):
            lo, hi = GR * gi, GR * (gi + 1)
            proj[gi] = (_dot_nt(wt2[D + 16 + lo:D + 16 + hi, :], xt), first[lo:hi])

        def vpu(gi):
            pq_t, q_t = proj.pop(gi)
            for i in range(GP):
                p = GP * gi + i
                phi = _feature_softmax(pq_t[40 * i:40 * (i + 1)]).astype(BF16)
                nd = _dot(lmat[p, :, 0:80], phi)
                rr = _seg_bcast((1.0 - g) * _recip(nd[40:41] + 1e-6), (1.0 - g) * _recip(nd[41:42] + 1e-6), low)
                ob = jnp.concatenate([a * b for a, b in zip(_tiles(nd[0:40]), rr)], axis=0)
                ot[D + 40 * p:D + 40 * (p + 1), cols] = ob.astype(BF16)
                kcp = kcol[40 * p:40 * (p + 1), :]
                for t in range(4):
                    tc = pl.ds(r0 + 128 * t, 128)
                    z = _tiles(q_t[40 * i:40 * (i + 1), 128 * t:128 * (t + 1)] * kcp)
                    az = [jnp.abs(a) for a in z]
                    m_a, m_b = _seg_reduce(az, jnp.maximum, jnp.max, 0.0, low1)
                    m_a = jnp.maximum(m_a, TINY)
                    m_b = jnp.maximum(m_b, TINY)
                    inv = _seg_bcast(FS * _recip(m_a), FS * _recip(m_b), low1)
                    bits = [lax.bitcast_convert_type(a * s_ + MAGIC, I32) for a, s_ in zip(z, inv)]
                    x0 = [(u << 20) >> 28 for u in bits]
                    x1 = [((u >> 4) & 15) - 8 for u in bits]
                    x2 = [(u & 15) - 8 for u in bits]
                    slots = [[a << 4 for a in x0], [a << 2 for a in x0], [a << 2 for a in x1], x1, x0, x2]
                    sig_a = m_a * (256.0 / (FS * FS))
                    sig_b = m_b * (256.0 / (FS * FS))
                    blk_a, blk_b = _head_blocks(slots, low1, shift_q, shift_q)
                    q8t[2 * p, :, tc] = blk_a.astype(I8)
                    q8t[2 * p + 1, :, tc] = blk_b.astype(I8)
                    sc[2 * p, :, tc] = jnp.broadcast_to(sig_a, (8, 128))
                    sc[2 * p + 1, :, tc] = jnp.broadcast_to(sig_b, (8, 128))
                    state["ok"] = jnp.minimum(
                        state["ok"], jnp.where(jnp.logical_and(m_a <= Q_MAX, m_b <= Q_MAX), 1.0, 0.0))

        mxu(0)
        for gi in range(NG):
            if gi + 1 < NG:
                mxu(gi + 1)
            vpu(gi)
        chk[0:1, :] = jnp.minimum(chk[0:1, :], state["ok"])
        return carry

    lax.fori_loop(0, NTS, phase2, 0)

    vmax = jnp.max(chk[8:16, :])
    fast = jnp.logical_and(jnp.min(chk[0:8, :]) > 0.5, jnp.logical_and(vmax >= V_MIN, vmax <= V_MAX))

    def finish_pair(p, acc_a, acc_b, cols, n):
        low = _lower(n)
        g = g_v[0:1, cols]
        ra = g * _recip(acc_a[20:21])
        rb = g * _recip(acc_b[16:17])
        o = jnp.concatenate([acc_a[0:8] * ra, acc_a[8:16] * ra,
                             jnp.where(low, acc_a[16:24] * ra, acc_b[16:24] * rb),
                             acc_b[0:8] * rb, acc_b[8:16] * rb], axis=0)
        ot[pl.ds(pl.multiple_of(40 * p, 8), 40), cols] = o.astype(BF16)

    @pl.when(fast)
    def _():
        nq = S // TQ
        nt = TQ // 128
        nch = S // CH

        def pair_body(p, carry):
            steps = [(qi, u) for qi in range(nq) for u in range(2)]
            pv = {}
            acc = {}

            def stage_a(g):
                s, j = divmod(g, nch)
                qi, u = steps[s]
                h = 2 * p + u
                z = jnp.dot(k8[h, j * CH:(j + 1) * CH, :], q8t[h, :, qi * TQ:(qi + 1) * TQ],
                            preferred_element_type=I32)
                for t in range(nt):
                    c0 = qi * TQ + t * 128
                    sig = sc[h, 0:1, c0:c0 + 128]
                    pv[(g, t)] = jnp.exp2(z[:, t * 128:(t + 1) * 128].astype(F32) * sig)

            nsub = CH // CB

            def stage_b(g, i):
                s, j = divmod(g, nch)
                qi, u = steps[s]
                h = 2 * p + u
                r0 = j * CH + i * CB
                v = vt[h, :, r0:r0 + CB]
                ds = [_dot(v, pv[(g, t)][i * CB:(i + 1) * CB].astype(BF16))[0:24] for t in range(nt)]
                acc[s] = ds if (j == 0 and i == 0) else [a + b for a, b in zip(acc[s], ds)]
                if j == nch - 1 and i == nsub - 1 and u == 1:
                    for t in range(nt):
                        c0 = qi * TQ + t * 128
                        finish_pair(p, acc[s - 1][t], acc[s][t], pl.ds(c0, 128), 128)

            total = len(steps) * nch
            seq = [(g, i) for g in range(total) for i in range(nsub)]
            done = 0
            for g in range(total):
                stage_a(g)
                while done < (g + 1) * nsub - SK:
                    stage_b(*seq[done])
                    done += 1
            while done < len(seq):
                stage_b(*seq[done])
                done += 1
            return carry

        lax.fori_loop(0, NP, pair_body, 0)

    @pl.when(jnp.logical_not(fast))
    def _():
        def proj(j, carry):
            cols = pl.ds(pl.multiple_of(j * TS, TS), TS)
            xt = x_v[cols, :]
            kt[:, cols] = _dot_nt(wt1[0:D, :], xt)
            qtf[:, cols] = _dot_nt(wt2[0:D, :], xt) * QSCALE
            return carry

        lax.fori_loop(0, NTS, proj, 0)
        tf = 256

        def body(i, carry):
            p = i // (S // tf)
            cols = pl.ds(pl.multiple_of((i % (S // tf)) * tf, tf), tf)
            rows = pl.ds(pl.multiple_of(40 * p, 8), 40)
            kp = kt[rows, :].astype(BF16)
            qp = qtf[rows, cols]
            first = lax.broadcasted_iota(I32, (40, tf), 0) < 20
            accs = []
            for u in range(2):
                qm = jnp.where(first if u == 0 else jnp.logical_not(first), qp, 0.0).astype(BF16)
                s_t = lax.dot_general(kp, qm, TN_DIMS, preferred_element_type=F32)
                pr = jnp.exp2(s_t - jnp.max(s_t, axis=0, keepdims=True)).astype(BF16)
                accs.append(_dot(vt[2 * p + u], pr)[0:24])
            finish_pair(p, accs[0], accs[1], cols, tf)
            return carry

        lax.fori_loop(0, NP * (S // tf), body, 0)

    def out_copy(j):
        return pltpu.make_async_copy(ostage.at[j % 2], out_hbm.at[0, pl.ds(j * TS, TS), :], out_sems.at[j % 2])

    for j in range(NTS):
        o_t = _dot(wot[...], ot[:, j * TS:(j + 1) * TS])
        if j >= 2:
            out_copy(j - 2).wait()
        ostage[j % 2] = o_t.T.astype(BF16)
        out_copy(j).start()
    out_copy(NTS - 2).wait()
    out_copy(NTS - 1).wait()


def _build():
    any_spec = pl.BlockSpec(memory_space=pl.ANY)
    scratch = [
        pltpu.VMEM((S, D), BF16),
        pltpu.VMEM((S, D), BF16),
        pltpu.VMEM((D, D), BF16),
        pltpu.VMEM((D, 2 * D), BF16),
        pltpu.VMEM((D, 3 * D), BF16),
        pltpu.VMEM((2 * D, D), BF16),
        pltpu.VMEM((D, 2 * D), BF16),
        pltpu.VMEM((DH, DH, H), BF16),
        pltpu.VMEM((D, 128), F32),
        pltpu.VMEM((D,), BF16),
        pltpu.VMEM((3 * D, D), BF16),
        pltpu.VMEM((3 * D + 16, D), BF16),
        pltpu.VMEM((5, TS, 128), F32),
        pltpu.VMEM((D, S), F32),
        pltpu.VMEM((D, 128), F32),
        pltpu.VMEM((D, 128), F32),
        pltpu.VMEM((NP, 48, 128), F32),
        pltpu.VMEM((NP, 48, 128), BF16),
        pltpu.VMEM((H, 128, S), I8),
        pltpu.VMEM((H, S, 128), I8),
        pltpu.VMEM((H, 32, S), BF16),
        pltpu.VMEM((H, 8, S), F32),
        pltpu.VMEM((8, S), F32),
        pltpu.VMEM((2 * D, S), BF16),
        pltpu.VMEM((2, TS, D), BF16),
        pltpu.VMEM((16, 128), F32),
        pltpu.VMEM((D, S), F32),
        pltpu.SemaphoreType.DMA((12,)),
        pltpu.SemaphoreType.DMA((2,)),
    ]
    return pl.pallas_call(
        _kernel,
        out_shape=jax.ShapeDtypeStruct((1, S, D), BF16),
        in_specs=[any_spec] * 7,
        out_specs=any_spec,
        scratch_shapes=scratch,
        compiler_params=pltpu.CompilerParams(vmem_limit_bytes=100 * 1024 * 1024),
        name="gated_mix_attn",
    )


@jax.jit
def pallas_gated_mix__mha_block__linear_kernel_hedgehog__prompt_kernel(
    A_x: jax.Array,
    A_wqkv: jax.Array,
    A_wo: jax.Array,
    B_x: jax.Array,
    B_wqkv: jax.Array,
    B_w_phi: jax.Array,
    B_wo: jax.Array,
    gate_w: jax.Array,
):
    del B_x
    w_phi = jnp.transpose(B_w_phi, (1, 2, 0))
    return _build()(A_x, A_wqkv, A_wo, B_wqkv, w_phi, B_wo, gate_w)
```

```python
import jax
import jax.numpy as jnp
from jax import lax
import jax.experimental.pallas as pl
import jax.experimental.pallas.tpu as pltpu

F32 = jnp.float32
BF16 = jnp.bfloat16
I32 = jnp.int32
U32 = jnp.uint32
I8 = jnp.int8

S = 2048
D = 640
H = 32
DH = 20
NP = H // 2
TS = 512
NTS = S // TS
GP = 16
GR = 40 * GP
NG = NP // GP
LOG2E = 1.4426950408889634
QSCALE = (DH ** -0.5) * LOG2E
FS = 1911.0
MAGIC = 12582912.0 + 136.0
TINY = 1e-30
Q_MAX = 3.5
V_MIN = 2.0 ** -16
V_MAX = 2.0 ** 60

NT_DIMS = (((1,), (1,)), ((), ()))
TN_DIMS = (((0,), (0,)), ((), ()))

TQ = 512
CH = 256
CB = 128
OU = 4
PB = 2
SK = 2


def _dot(a, b):
    return jnp.dot(a, b, preferred_element_type=F32)


def _dot_nt(a, b):
    return lax.dot_general(a, b, NT_DIMS, preferred_element_type=F32)


def _recip(x):
    r = pl.reciprocal(x, approx=True)
    return r * (2.0 - x * r)


def _lower(n):
    return lax.broadcasted_iota(I32, (8, n), 0) < 4


def _seg_reduce(v, op, red, fill, low):
    a = op(op(v[0], v[1]), jnp.where(low, v[2], fill))
    b = op(op(v[3], v[4]), jnp.where(low, fill, v[2]))
    return red(a, axis=0, keepdims=True), red(b, axis=0, keepdims=True)


def _seg_bcast(a, b, low):
    n = a.shape[-1]
    a8 = jnp.broadcast_to(a, (8, n))
    b8 = jnp.broadcast_to(b, (8, n))
    return [a8, a8, jnp.where(low, a8, b8), b8, b8]


def _tiles(z):
    return [z[8 * i:8 * (i + 1)] for i in range(z.shape[0] // 8)]


def _feature_softmax(z):
    n = z.shape[-1]
    low = _lower(n)
    v = _tiles(z)
    mx = _seg_bcast(*_seg_reduce(v, jnp.maximum, jnp.max, -jnp.inf, low), low)
    mn = _seg_bcast(*_seg_reduce(v, jnp.minimum, jnp.min, jnp.inf, low), low)
    ep = [jnp.exp2(a - m) for a, m in zip(v, mx)]
    en = [jnp.exp2(m - a) for a, m in zip(v, mn)]
    sa, sb = _seg_reduce(ep, jnp.add, jnp.sum, 0.0, low)
    rp = _seg_bcast(_recip(sa), _recip(sb), low)
    sa, sb = _seg_reduce(en, jnp.add, jnp.sum, 0.0, low)
    rn = _seg_bcast(_recip(sa), _recip(sb), low)
    return jnp.concatenate([e * r for e, r in zip(ep, rp)] + [e * r for e, r in zip(en, rn)], axis=0)


def _head_blocks(slots, low, last_a, last_b):
    blk_a, blk_b = [], []
    for t in range(6):
        blk_a += [slots[t][0], slots[t][1]]
        blk_b += [slots[t][3], slots[t][4]]
    for t in range(0, 6, 2):
        lo, hi = slots[t][2], slots[t + 1][2]
        blk_a.append(jnp.where(low, lo, pltpu.roll(hi, 4, 0)))
        blk_b.append(jnp.where(low, pltpu.roll(lo, 4, 0), hi))
    blk_a.append(last_a)
    blk_b.append(last_b)
    return jnp.concatenate(blk_a, axis=0), jnp.concatenate(blk_b, axis=0)


def _kernel(x_hbm, wa_hbm, woa_hbm, wb_hbm, wphi_hbm, wob_hbm, gate_hbm, out_hbm,
            x_v, xp_v, wak_v, waqv_v, wb_v, wo_v, wot, wphi_v, w2s, gate_v, wt1, wt2, xs, kt, kcol, kinv_v, kv, lmat,
            q8t, k8, vt, sc, g_v, ot, ostage, chk, qtf, in_sems, out_sems):
    cp_x = [pltpu.make_async_copy(x_hbm.at[0, pl.ds(j * TS, TS), :], x_v.at[pl.ds(j * TS, TS), :], in_sems.at[j])
            for j in range(NTS)]
    cp_wk = pltpu.make_async_copy(wa_hbm.at[:, pl.ds(D, D)], wak_v, in_sems.at[4])
    cp_wb = pltpu.make_async_copy(wb_hbm, wb_v, in_sems.at[5])
    cp_phi = pltpu.make_async_copy(wphi_hbm, wphi_v, in_sems.at[6])
    cp_gate = pltpu.make_async_copy(gate_hbm, gate_v, in_sems.at[7])
    cp_wq = pltpu.make_async_copy(wa_hbm.at[:, pl.ds(0, D)], waqv_v.at[:, pl.ds(0, D)], in_sems.at[8])
    cp_wv = pltpu.make_async_copy(wa_hbm.at[:, pl.ds(2 * D, D)], waqv_v.at[:, pl.ds(D, D)], in_sems.at[9])
    cp_woa = pltpu.make_async_copy(woa_hbm, wo_v.at[0:D], in_sems.at[10])
    cp_wob = pltpu.make_async_copy(wob_hbm, wo_v.at[D:2 * D], in_sems.at[11])
    for c in (cp_x[0], cp_wk, cp_x[1], cp_x[2], cp_x[3], cp_wb, cp_phi, cp_gate):
        c.start()
    chk[...] = jnp.concatenate([jnp.ones((8, 128), F32), jnp.zeros((8, 128), F32)], axis=0)

    def permute(j):
        r0 = j * TS
        for c in range(5):
            xs[c] = x_v[r0:r0 + TS, 128 * c:128 * (c + 1)].astype(F32)
        for b in range(4):
            xp_v[r0 + 128 * b:r0 + 128 * (b + 1), :] = jnp.concatenate(
                [xs[c, pl.ds(b, 128, stride=4), :] for c in range(5)], axis=1).astype(BF16)

    def keys(j):
        r0 = j * TS
        k_t = _dot_nt(wt1[0:D, :], xp_v[r0:r0 + TS, :])
        kt[:, r0:r0 + TS] = k_t
        ak = jnp.abs(k_t)
        m = ak[:, 0:128]
        fin = ak[:, 0:128] < jnp.inf
        for b in range(1, 4):
            m = jnp.maximum(m, ak[:, 128 * b:128 * (b + 1)])
            fin = jnp.logical_and(fin, ak[:, 128 * b:128 * (b + 1)] < jnp.inf)
        kcol[...] = m if j == 0 else jnp.maximum(kcol[...], m)
        okf = jnp.min(jnp.where(fin, 1.0, 0.0).reshape(D // 8, 8, 128), axis=0)
        chk[0:8, :] = jnp.minimum(chk[0:8, :], okf)

    cp_x[0].wait()
    permute(0)
    cp_wk.wait()
    cp_x[1].wait()
    wt1[0:D, :] = wak_v[...].T
    keys(0)
    permute(1)
    cp_x[2].wait()
    cp_x[3].wait()
    cp_wv.start()
    cp_wq.start()
    permute(2)
    keys(1)
    permute(3)
    keys(2)
    cp_wb.wait()
    cp_phi.wait()
    cp_gate.wait()
    cp_wv.wait()
    keys(3)
    kv[...] = jnp.zeros_like(kv)
    wt2[2 * D + 16:3 * D + 16, :] = waqv_v[:, D:2 * D].T
    wt1[2 * D:3 * D, :] = wb_v[:, 2 * D:3 * D].T
    for blk in range(5):
        rows = []
        for dl in range(4):
            a = wphi_v[4 * blk + dl].astype(F32)
            rows += [jnp.concatenate([a, jnp.zeros((DH, 128 - H), F32)], axis=1), jnp.zeros((12, 128), F32)]
        t = jnp.concatenate(rows, axis=0).T[0:H]
        for dl in range(4):
            w2s[pl.ds(4 * blk + dl, H, stride=DH), :] = t if dl == 0 else pltpu.roll(t, 128 - 32 * dl, 1)
    w2t = w2s[...].T.astype(BF16)
    for i, (k0, k1) in enumerate(((0, 2), (0, 3), (1, 4), (2, 5), (3, 5))):
        rows = lax.broadcasted_iota(I32, (128, 128), 0) + 128 * i
        sel = (rows % DH == lax.broadcasted_iota(I32, (128, 128), 1)).astype(BF16)
        rep = _dot(sel, w2t[:, 128 * k0:128 * k1])
        rh = rows // DH
        blk = []
        for k in range(k0, k1):
            ch = (lax.broadcasted_iota(I32, (8, 128), 1) + 128 * k) // DH
            blk.append(jnp.where(rh == ch[0:1], rep[:, 128 * (k - k0):128 * (k - k0 + 1)], 0.0))
        bdt = jnp.concatenate(blk, axis=1).astype(BF16)
        wt1[D + 128 * i:D + 128 * (i + 1), :] = (
            _dot_nt(bdt, wb_v[:, D + 128 * k0:D + 128 * k1]) * LOG2E).astype(BF16)
        wt2[D + 16 + 128 * i:D + 16 + 128 * (i + 1), :] = (
            _dot_nt(bdt, wb_v[:, 128 * k0:128 * k1]) * LOG2E).astype(BF16)
    grow = jnp.broadcast_to(gate_v[...].astype(F32).reshape(1, D), (16, D))
    wt2[D:D + 16, :] = grow.astype(BF16)
    kc = jnp.maximum(jnp.max(kcol[...], axis=1, keepdims=True), TINY)
    kinv_v[...] = jnp.broadcast_to(FS / kc, (D, 128))
    kcol[...] = jnp.broadcast_to(kc * QSCALE, (D, 128))
    cp_woa.start()
    cp_wob.start()
    cp_wq.wait()

    def key_digits(p, r0, cols, low1):
        kinv = kinv_v[40 * p:40 * (p + 1), :]
        w0 = w1 = w2_ = None
        for b in range(4):
            y = kt[40 * p:40 * (p + 1), pl.ds(r0 + 128 * b, 128)] * kinv + MAGIC
            u = lax.bitcast_convert_type(y, U32)
            msk = jnp.uint32(15 << (8 * b))
            n2 = (u << (8 * b)) & msk
            n1 = ((u >> 4) if b == 0 else (u << (8 * b - 4))) & msk
            n0 = ((u >> 8) if b == 0 else (u if b == 1 else (u << (8 * b - 8)))) & msk
            w0 = n0 if b == 0 else w0 | n0
            w1 = n1 if b == 0 else w1 | n1
            w2_ = n2 if b == 0 else w2_ | n2
        c78 = jnp.uint32(0x78787878)
        c80 = jnp.uint32(0x80808080)
        w0 = ((w0 ^ jnp.uint32(0x08080808)) + c78) ^ c80
        w1 = (w1 + c78) ^ c80
        w2_ = (w2_ + c78) ^ c80
        cf0 = jnp.uint32(0xF0F0F0F0)
        cfc = jnp.uint32(0xFCFCFCFC)
        slots = [_tiles((w0 << 4) & cf0), _tiles((w1 << 2) & cfc), _tiles((w0 << 2) & cfc),
                 _tiles(w1), _tiles(w2_), _tiles(w0)]
        shift_w = jnp.where(lax.broadcasted_iota(I32, (8, 128), 0) == 0,
                            jnp.uint32(0xFFFFFFFF), jnp.uint32(0x80808080))
        blk_a, blk_b = _head_blocks(slots, low1, shift_w, shift_w)
        k8[2 * p, cols, :] = pltpu.bitcast(lax.bitcast_convert_type(blk_a, I32).T, I8)
        k8[2 * p + 1, cols, :] = pltpu.bitcast(lax.bitcast_convert_type(blk_b, I32).T, I8)

    def phase1(j, carry):
        r0 = pl.multiple_of(j * TS, TS)
        cols = pl.ds(r0, TS)
        xt = x_v[cols, :]
        ones8 = jnp.where(lax.broadcasted_iota(I32, (8, TS), 0) == 0, 1.0, 0.0)
        low1 = _lower(128)
        low = _lower(TS)
        sub = lax.broadcasted_iota(I32, (8, TS), 0)
        zero8 = jnp.zeros((8, TS), F32)
        proj = {}
        state = {"vm": jnp.zeros((8, TS), F32)}

        def mxu(g):
            lo, hi = GR * g, GR * (g + 1)
            proj[g] = (_dot_nt(wt1[D + lo:D + hi, :], xt), _dot_nt(wt1[2 * D + lo:2 * D + hi, :], xt),
                       _dot_nt(wt2[2 * D + 16 + lo:2 * D + 16 + hi, :], xt))

        def vpu(g):
            pk_t, vb_t, va_t = proj.pop(g)
            for i in range(GP):
                p = GP * g + i
                v = _tiles(va_t[40 * i:40 * (i + 1)])
                for a in v:
                    state["vm"] = jnp.maximum(state["vm"], jnp.abs(a))
                mid_a = jnp.where(low, v[2], jnp.where(sub == 4, 1.0, 0.0))
                mid_b = jnp.where(low, jnp.where(sub == 0, 1.0, 0.0), v[2])
                vt[2 * p, :, cols] = jnp.concatenate([v[0], v[1], mid_a, zero8], axis=0).astype(BF16)
                vt[2 * p + 1, :, cols] = jnp.concatenate([v[3], v[4], mid_b, zero8], axis=0).astype(BF16)
                phi = _feature_softmax(pk_t[40 * i:40 * (i + 1)]).astype(BF16)
                vaug = jnp.concatenate([vb_t[40 * i:40 * (i + 1)], ones8], axis=0).astype(BF16)
                kv[p, :, 0:80] = kv[p, :, 0:80] + _dot_nt(vaug, phi)
                key_digits(p, r0, cols, low1)

        for i in range(2):
            r = pl.multiple_of(jnp.minimum(2 * j + i, 4) * 128, 128)
            wt2[pl.ds(r, 128), :] = waqv_v[:, pl.ds(r, 128)].T
        mxu(0)
        for g in range(NG):
            if g + 1 < NG:
                mxu(g + 1)
            vpu(g)
        vm = state["vm"]
        for b in range(4):
            chk[8:16, :] = jnp.maximum(chk[8:16, :], vm[:, 128 * b:128 * (b + 1)])
        return carry

    lax.fori_loop(0, NTS, phase1, 0)

    kvv = kv[...]
    r = lax.broadcasted_iota(I32, (NP, 48, 128), 1)
    c = lax.broadcasted_iota(I32, (NP, 48, 128), 2)
    col_a = (c < 20) | ((c >= 40) & (c < 60))
    col_b = ((c >= 20) & (c < 40)) | ((c >= 60) & (c < 80))
    row_a = (r < 20) | (r == 40)
    row_b = ((r >= 20) & (r < 40)) | (r == 41)
    src = jnp.where(r >= 40, jnp.broadcast_to(kvv[:, 40:41, :], (NP, 48, 128)), kvv)
    lmat[...] = jnp.where((row_a & col_a) | (row_b & col_b), src, 0.0).astype(BF16)

    cp_woa.wait()
    cp_wob.wait()

    def phase2(j, carry):
        r0 = pl.multiple_of(j * TS, TS)
        cols = pl.ds(r0, TS)
        xt = x_v[cols, :]
        for i in range(3):
            r = pl.multiple_of(jnp.minimum(3 * j + i, 9) * 128, 128)
            wot[:, pl.ds(r, 128)] = wo_v[pl.ds(r, 128), :].T
        first = _dot_nt(wt2[0:D + 16, :], xt)
        g = jax.nn.sigmoid(first[D:D + 1])
        g_v[:, cols] = jnp.broadcast_to(g, (8, TS))
        low = _lower(TS)
        low1 = _lower(128)
        shift_q = jnp.full((8, 128), 127, I32)
        proj = {}
        state = {"ok": jnp.ones((1, 128), F32)}

        def mxu(gi):
            lo, hi = GR * gi, GR * (gi + 1)
            proj[gi] = (_dot_nt(wt2[D + 16 + lo:D + 16 + hi, :], xt), first[lo:hi])

        def vpu(gi):
            pq_t, q_t = proj.pop(gi)
            for i in range(GP):
                p = GP * gi + i
                phi = _feature_softmax(pq_t[40 * i:40 * (i + 1)]).astype(BF16)
                nd = _dot(lmat[p, :, 0:80], phi)
                rr = _seg_bcast((1.0 - g) * _recip(nd[40:41] + 1e-6), (1.0 - g) * _recip(nd[41:42] + 1e-6), low)
                ob = jnp.concatenate([a * b for a, b in zip(_tiles(nd[0:40]), rr)], axis=0)
                ot[D + 40 * p:D + 40 * (p + 1), cols] = ob.astype(BF16)
                kcp = kcol[40 * p:40 * (p + 1), :]
                for t in range(4):
                    tc = pl.ds(r0 + 128 * t, 128)
                    z = _tiles(q_t[40 * i:40 * (i + 1), 128 * t:128 * (t + 1)] * kcp)
                    az = [jnp.abs(a) for a in z]
                    m_a, m_b = _seg_reduce(az, jnp.maximum, jnp.max, 0.0, low1)
                    m_a = jnp.maximum(m_a, TINY)
                    m_b = jnp.maximum(m_b, TINY)
                    inv = _seg_bcast(FS * _recip(m_a), FS * _recip(m_b), low1)
                    bits = [lax.bitcast_convert_type(a * s_ + MAGIC, I32) for a, s_ in zip(z, inv)]
                    x0 = [(u << 20) >> 28 for u in bits]
                    x1 = [((u >> 4) & 15) - 8 for u in bits]
                    x2 = [(u & 15) - 8 for u in bits]
                    slots = [[a << 4 for a in x0], [a << 2 for a in x0], [a << 2 for a in x1], x1, x0, x2]
                    sig_a = m_a * (256.0 / (FS * FS))
                    sig_b = m_b * (256.0 / (FS * FS))
                    blk_a, blk_b = _head_blocks(slots, low1, shift_q, shift_q)
                    q8t[2 * p, :, tc] = blk_a.astype(I8)
                    q8t[2 * p + 1, :, tc] = blk_b.astype(I8)
                    sc[2 * p, :, tc] = jnp.broadcast_to(sig_a, (8, 128))
                    sc[2 * p + 1, :, tc] = jnp.broadcast_to(sig_b, (8, 128))
                    state["ok"] = jnp.minimum(
                        state["ok"], jnp.where(jnp.logical_and(m_a <= Q_MAX, m_b <= Q_MAX), 1.0, 0.0))

        mxu(0)
        for gi in range(NG):
            if gi + 1 < NG:
                mxu(gi + 1)
            vpu(gi)
        chk[0:1, :] = jnp.minimum(chk[0:1, :], state["ok"])
        return carry

    lax.fori_loop(0, NTS, phase2, 0)

    vmax = jnp.max(chk[8:16, :])
    fast = jnp.logical_and(jnp.min(chk[0:8, :]) > 0.5, jnp.logical_and(vmax >= V_MIN, vmax <= V_MAX))

    def finish_pair(p, acc_a, acc_b, cols, n):
        low = _lower(n)
        g = g_v[0:1, cols]
        ra = g * _recip(acc_a[20:21])
        rb = g * _recip(acc_b[16:17])
        o = jnp.concatenate([acc_a[0:8] * ra, acc_a[8:16] * ra,
                             jnp.where(low, acc_a[16:24] * ra, acc_b[16:24] * rb),
                             acc_b[0:8] * rb, acc_b[8:16] * rb], axis=0)
        ot[pl.ds(pl.multiple_of(40 * p, 8), 40), cols] = o.astype(BF16)

    @pl.when(fast)
    def _():
        nq = S // TQ
        nt = TQ // 128
        nch = S // CH

        def pair_body(pb, carry):
            steps = [(qi, u) for pp in range(PB) for qi in range(nq) for u in range(2 * pp, 2 * pp + 2)]
            pv = {}
            acc = {}

            def stage_a(g):
                s, j = divmod(g, nch)
                qi, u = steps[s]
                h = 2 * PB * pb + u
                z = jnp.dot(k8[h, j * CH:(j + 1) * CH, :], q8t[h, :, qi * TQ:(qi + 1) * TQ],
                            preferred_element_type=I32)
                for t in range(nt):
                    c0 = qi * TQ + t * 128
                    sig = sc[h, 0:1, c0:c0 + 128]
                    pv[(g, t)] = jnp.exp2(z[:, t * 128:(t + 1) * 128].astype(F32) * sig)

            nsub = CH // CB

            def stage_b(g, i):
                s, j = divmod(g, nch)
                qi, u = steps[s]
                h = 2 * PB * pb + u
                r0 = j * CH + i * CB
                v = vt[h, :, r0:r0 + CB]
                ds = [_dot(v, pv[(g, t)][i * CB:(i + 1) * CB].astype(BF16))[0:24] for t in range(nt)]
                acc[s] = ds if (j == 0 and i == 0) else [a + b for a, b in zip(acc[s], ds)]
                if j == nch - 1 and i == nsub - 1 and u % 2 == 1:
                    for t in range(nt):
                        c0 = qi * TQ + t * 128
                        finish_pair(PB * pb + u // 2, acc[s - 1][t], acc[s][t], pl.ds(c0, 128), 128)

            total = len(steps) * nch
            seq = [(g, i) for g in range(total) for i in range(nsub)]
            done = 0
            for g in range(total):
                stage_a(g)
                while done < (g + 1) * nsub - SK:
                    stage_b(*seq[done])
                    done += 1
            while done < len(seq):
                stage_b(*seq[done])
                done += 1
            return carry

        lax.fori_loop(0, NP // PB, pair_body, 0)

    @pl.when(jnp.logical_not(fast))
    def _():
        def proj(j, carry):
            cols = pl.ds(pl.multiple_of(j * 128, 128), 128)
            xt = x_v[cols, :]
            kt[:, cols] = _dot_nt(wt1[0:D, :], xt)
            qtf[:, cols] = _dot_nt(wt2[0:D, :], xt) * QSCALE
            return carry

        lax.fori_loop(0, S // 128, proj, 0)
        tf = 128

        def body(i, carry):
            p = i // (S // tf)
            cols = pl.ds(pl.multiple_of((i % (S // tf)) * tf, tf), tf)
            rows = pl.ds(pl.multiple_of(40 * p, 8), 40)
            kp = kt[rows, :].astype(BF16)
            qp = qtf[rows, cols]
            first = lax.broadcasted_iota(I32, (40, tf), 0) < 20
            accs = []
            for u in range(2):
                qm = jnp.where(first if u == 0 else jnp.logical_not(first), qp, 0.0).astype(BF16)
                s_t = lax.dot_general(kp, qm, TN_DIMS, preferred_element_type=F32)
                pr = jnp.exp2(s_t - jnp.max(s_t, axis=0, keepdims=True)).astype(BF16)
                accs.append(_dot(vt[2 * p + u], pr)[0:24])
            finish_pair(p, accs[0], accs[1], cols, tf)
            return carry

        lax.fori_loop(0, NP * (S // tf), body, 0)

    def out_copy(j):
        rows = pl.ds(pl.multiple_of(j * TS, TS), TS)
        return pltpu.make_async_copy(ostage.at[j], out_hbm.at[0, rows, :], out_sems.at[j])

    def out_body(i, carry):
        for u in range(OU):
            j = OU * i + u
            o_t = _dot(wot[...], ot[:, pl.ds(pl.multiple_of(j * TS, TS), TS)])
            ostage[j] = o_t.T.astype(BF16)
            out_copy(j).start()
        return carry

    lax.fori_loop(0, NTS // OU, out_body, 0)
    for j in range(NTS):
        out_copy(j).wait()


def _build():
    any_spec = pl.BlockSpec(memory_space=pl.ANY)
    scratch = [
        pltpu.VMEM((S, D), BF16),
        pltpu.VMEM((S, D), BF16),
        pltpu.VMEM((D, D), BF16),
        pltpu.VMEM((D, 2 * D), BF16),
        pltpu.VMEM((D, 3 * D), BF16),
        pltpu.VMEM((2 * D, D), BF16),
        pltpu.VMEM((D, 2 * D), BF16),
        pltpu.VMEM((DH, DH, H), BF16),
        pltpu.VMEM((D, 128), F32),
        pltpu.VMEM((D,), BF16),
        pltpu.VMEM((3 * D, D), BF16),
        pltpu.VMEM((3 * D + 16, D), BF16),
        pltpu.VMEM((5, TS, 128), F32),
        pltpu.VMEM((D, S), F32),
        pltpu.VMEM((D, 128), F32),
        pltpu.VMEM((D, 128), F32),
        pltpu.VMEM((NP, 48, 128), F32),
        pltpu.VMEM((NP, 48, 128), BF16),
        pltpu.VMEM((H, 128, S), I8),
        pltpu.VMEM((H, S, 128), I8),
        pltpu.VMEM((H, 32, S), BF16),
        pltpu.VMEM((H, 8, S), F32),
        pltpu.VMEM((8, S), F32),
        pltpu.VMEM((2 * D, S), BF16),
        pltpu.VMEM((NTS, TS, D), BF16),
        pltpu.VMEM((16, 128), F32),
        pltpu.VMEM((D, S), F32),
        pltpu.SemaphoreType.DMA((12,)),
        pltpu.SemaphoreType.DMA((NTS,)),
    ]
    return pl.pallas_call(
        _kernel,
        out_shape=jax.ShapeDtypeStruct((1, S, D), BF16),
        in_specs=[any_spec] * 7,
        out_specs=any_spec,
        scratch_shapes=scratch,
        compiler_params=pltpu.CompilerParams(vmem_limit_bytes=100 * 1024 * 1024),
        name="gated_mix_attn",
    )


@jax.jit
def pallas_gated_mix__mha_block__linear_kernel_hedgehog__prompt_kernel(
    A_x: jax.Array,
    A_wqkv: jax.Array,
    A_wo: jax.Array,
    B_x: jax.Array,
    B_wqkv: jax.Array,
    B_w_phi: jax.Array,
    B_wo: jax.Array,
    gate_w: jax.Array,
):
    del B_x
    w_phi = jnp.transpose(B_w_phi, (1, 2, 0))
    return _build()(A_x, A_wqkv, A_wo, B_wqkv, w_phi, B_wo, gate_w)
```

```python
import jax
import jax.numpy as jnp
from jax import lax
import jax.experimental.pallas as pl
import jax.experimental.pallas.tpu as pltpu

F32 = jnp.float32
BF16 = jnp.bfloat16
I32 = jnp.int32
U32 = jnp.uint32
I8 = jnp.int8

S = 2048
D = 640
H = 32
DH = 20
NP = H // 2
TS = 512
NTS = S // TS
GP = 16
GR = 40 * GP
NG = NP // GP
LOG2E = 1.4426950408889634
QSCALE = (DH ** -0.5) * LOG2E
FS = 1911.0
MAGIC = 12582912.0 + 136.0
TINY = 1e-30
Q_MAX = 3.5
V_MIN = 2.0 ** -16
V_MAX = 2.0 ** 60

NT_DIMS = (((1,), (1,)), ((), ()))
TN_DIMS = (((0,), (0,)), ((), ()))

TQ = 512
CH = 128
CB = 128
AG = 2
PB = 2
SK = 2


def _dot(a, b):
    return jnp.dot(a, b, preferred_element_type=F32)


def _dot_nt(a, b):
    return lax.dot_general(a, b, NT_DIMS, preferred_element_type=F32)


def _recip(x):
    r = pl.reciprocal(x, approx=True)
    return r * (2.0 - x * r)


def _transpose_into(dst, row0, src, col0, ncols):
    for c in range(0, ncols, 128):
        dst[row0 + c:row0 + c + 128, :] = src[:, col0 + c:col0 + c + 128].T


def _lower(n):
    return lax.broadcasted_iota(I32, (8, n), 0) < 4


def _seg_reduce(v, op, red, fill, low):
    a = op(op(v[0], v[1]), jnp.where(low, v[2], fill))
    b = op(op(v[3], v[4]), jnp.where(low, fill, v[2]))
    return red(a, axis=0, keepdims=True), red(b, axis=0, keepdims=True)


def _seg_bcast(a, b, low):
    n = a.shape[-1]
    a8 = jnp.broadcast_to(a, (8, n))
    b8 = jnp.broadcast_to(b, (8, n))
    return [a8, a8, jnp.where(low, a8, b8), b8, b8]


def _tiles(z):
    return [z[8 * i:8 * (i + 1)] for i in range(z.shape[0] // 8)]


def _feature_softmax(z):
    n = z.shape[-1]
    low = _lower(n)
    v = _tiles(z)
    mx = _seg_bcast(*_seg_reduce(v, jnp.maximum, jnp.max, -jnp.inf, low), low)
    mn = _seg_bcast(*_seg_reduce(v, jnp.minimum, jnp.min, jnp.inf, low), low)
    ep = [jnp.exp2(a - m) for a, m in zip(v, mx)]
    en = [jnp.exp2(m - a) for a, m in zip(v, mn)]
    sa, sb = _seg_reduce(ep, jnp.add, jnp.sum, 0.0, low)
    rp = _seg_bcast(_recip(sa), _recip(sb), low)
    sa, sb = _seg_reduce(en, jnp.add, jnp.sum, 0.0, low)
    rn = _seg_bcast(_recip(sa), _recip(sb), low)
    return jnp.concatenate([e * r for e, r in zip(ep, rp)] + [e * r for e, r in zip(en, rn)], axis=0)


def _head_blocks(slots, low, last_a, last_b):
    blk_a, blk_b = [], []
    for t in range(6):
        blk_a += [slots[t][0], slots[t][1]]
        blk_b += [slots[t][3], slots[t][4]]
    for t in range(0, 6, 2):
        lo, hi = slots[t][2], slots[t + 1][2]
        blk_a.append(jnp.where(low, lo, pltpu.roll(hi, 4, 0)))
        blk_b.append(jnp.where(low, pltpu.roll(lo, 4, 0), hi))
    blk_a.append(last_a)
    blk_b.append(last_b)
    return jnp.concatenate(blk_a, axis=0), jnp.concatenate(blk_b, axis=0)


def _kernel(x_hbm, wa_hbm, woa_hbm, wb_hbm, wphi_hbm, wob_hbm, gate_hbm, out_hbm,
            x_v, xp_v, wak_v, waqv_v, wb_v, wbt, wo_v, wot, wphi_v, w2s, gate_v, wt1, wt2, xs, kt, kcol, kinv_v, kv, lmat,
            q8t, k8, vt, sc, g_v, ot, ostage, chk, qtf, in_sems, out_sems):
    cp_x = [pltpu.make_async_copy(x_hbm.at[0, pl.ds(j * TS, TS), :], x_v.at[pl.ds(j * TS, TS), :], in_sems.at[j])
            for j in range(NTS)]
    cp_wk = pltpu.make_async_copy(wa_hbm.at[:, pl.ds(D, D)], wak_v, in_sems.at[4])
    cp_wb = pltpu.make_async_copy(wb_hbm, wb_v, in_sems.at[5])
    cp_phi = pltpu.make_async_copy(wphi_hbm, wphi_v, in_sems.at[6])
    cp_gate = pltpu.make_async_copy(gate_hbm, gate_v, in_sems.at[7])
    cp_wq = pltpu.make_async_copy(wa_hbm.at[:, pl.ds(0, D)], waqv_v.at[:, pl.ds(0, D)], in_sems.at[8])
    cp_wv = pltpu.make_async_copy(wa_hbm.at[:, pl.ds(2 * D, D)], waqv_v.at[:, pl.ds(D, D)], in_sems.at[9])
    cp_woa = pltpu.make_async_copy(woa_hbm, wo_v.at[0:D], in_sems.at[10])
    cp_wob = pltpu.make_async_copy(wob_hbm, wo_v.at[D:2 * D], in_sems.at[11])
    for c in (cp_x[0], cp_wk, cp_x[1], cp_x[2], cp_x[3], cp_wb, cp_phi, cp_gate):
        c.start()
    chk[...] = jnp.concatenate([jnp.ones((8, 128), F32), jnp.zeros((8, 128), F32)], axis=0)

    def permute(j):
        r0 = j * TS
        for c in range(5):
            xs[c] = x_v[r0:r0 + TS, 128 * c:128 * (c + 1)].astype(F32)
        for b in range(4):
            xp_v[r0 + 128 * b:r0 + 128 * (b + 1), :] = jnp.concatenate(
                [xs[c, pl.ds(b, 128, stride=4), :] for c in range(5)], axis=1).astype(BF16)

    def keys(j):
        r0 = j * TS
        k_t = _dot_nt(wt1[0:D, :], xp_v[r0:r0 + TS, :])
        kt[:, r0:r0 + TS] = k_t
        ak = jnp.abs(k_t)
        m = ak[:, 0:128]
        fin = ak[:, 0:128] < jnp.inf
        for b in range(1, 4):
            m = jnp.maximum(m, ak[:, 128 * b:128 * (b + 1)])
            fin = jnp.logical_and(fin, ak[:, 128 * b:128 * (b + 1)] < jnp.inf)
        kcol[...] = m if j == 0 else jnp.maximum(kcol[...], m)
        okf = jnp.min(jnp.where(fin, 1.0, 0.0).reshape(D // 8, 8, 128), axis=0)
        chk[0:8, :] = jnp.minimum(chk[0:8, :], okf)

    cp_x[0].wait()
    permute(0)
    cp_wk.wait()
    cp_x[1].wait()
    _transpose_into(wt1, 0, wak_v, 0, D)
    keys(0)
    permute(1)
    cp_x[2].wait()
    cp_x[3].wait()
    cp_wv.start()
    cp_wq.start()
    permute(2)
    keys(1)
    permute(3)
    keys(2)
    cp_wb.wait()
    cp_phi.wait()
    cp_gate.wait()
    cp_wv.wait()
    _transpose_into(wbt, 0, wb_v, 0, 2 * D)
    keys(3)
    kv[...] = jnp.zeros_like(kv)
    for blk in range(5):
        rows = []
        for dl in range(4):
            a = wphi_v[4 * blk + dl].astype(F32)
            rows += [jnp.concatenate([a, jnp.zeros((DH, 128 - H), F32)], axis=1), jnp.zeros((12, 128), F32)]
        t = jnp.concatenate(rows, axis=0).T[0:H]
        for dl in range(4):
            w2s[pl.ds(4 * blk + dl, H, stride=DH), :] = t if dl == 0 else pltpu.roll(t, 128 - 32 * dl, 1)
    row = lax.broadcasted_iota(I32, (40, 128), 0)
    lane = lax.broadcasted_iota(I32, (40, 128), 1)
    for p in range(NP):
        a = w2s[40 * p:40 * (p + 1), :]
        m = jnp.where(row < DH, jnp.where(lane < DH, a, 0.0),
                      jnp.where((lane >= DH) & (lane < 2 * DH), pltpu.roll(a, DH, 1), 0.0))
        lhs = m.T[0:48].astype(BF16)
        rhs = jnp.concatenate([wbt[40 * p:40 * (p + 1), :], wbt[D + 40 * p:D + 40 * (p + 1), :]], axis=1)
        res = (_dot(lhs, rhs)[0:40] * LOG2E).astype(BF16)
        wt2[D + 16 + 40 * p:D + 16 + 40 * (p + 1), :] = res[:, 0:D]
        wt1[D + 40 * p:D + 40 * (p + 1), :] = res[:, D:2 * D]
    _transpose_into(wt1, 2 * D, wb_v, 2 * D, D)
    _transpose_into(wt2, 2 * D + 16, waqv_v, D, D)
    grow = jnp.broadcast_to(gate_v[...].astype(F32).reshape(1, D), (16, D))
    wt2[D:D + 16, :] = grow.astype(BF16)
    kc = jnp.maximum(jnp.max(kcol[...], axis=1, keepdims=True), TINY)
    kinv_v[...] = jnp.broadcast_to(FS / kc, (D, 128))
    kcol[...] = jnp.broadcast_to(kc * QSCALE, (D, 128))
    cp_woa.start()
    cp_wob.start()
    cp_wq.wait()

    def key_digits(p, r0, cols, low1):
        kinv = kinv_v[40 * p:40 * (p + 1), :]
        w0 = w1 = w2_ = None
        for b in range(4):
            y = kt[40 * p:40 * (p + 1), pl.ds(r0 + 128 * b, 128)] * kinv + MAGIC
            u = lax.bitcast_convert_type(y, U32)
            msk = jnp.uint32(15 << (8 * b))
            n2 = (u << (8 * b)) & msk
            n1 = ((u >> 4) if b == 0 else (u << (8 * b - 4))) & msk
            n0 = ((u >> 8) if b == 0 else (u if b == 1 else (u << (8 * b - 8)))) & msk
            w0 = n0 if b == 0 else w0 | n0
            w1 = n1 if b == 0 else w1 | n1
            w2_ = n2 if b == 0 else w2_ | n2
        c78 = jnp.uint32(0x78787878)
        c80 = jnp.uint32(0x80808080)
        w0 = ((w0 ^ jnp.uint32(0x08080808)) + c78) ^ c80
        w1 = (w1 + c78) ^ c80
        w2_ = (w2_ + c78) ^ c80
        cf0 = jnp.uint32(0xF0F0F0F0)
        cfc = jnp.uint32(0xFCFCFCFC)
        slots = [_tiles((w0 << 4) & cf0), _tiles((w1 << 2) & cfc), _tiles((w0 << 2) & cfc),
                 _tiles(w1), _tiles(w2_), _tiles(w0)]
        shift_w = jnp.where(lax.broadcasted_iota(I32, (8, 128), 0) == 0,
                            jnp.uint32(0xFFFFFFFF), jnp.uint32(0x80808080))
        blk_a, blk_b = _head_blocks(slots, low1, shift_w, shift_w)
        k8[2 * p, cols, :] = pltpu.bitcast(lax.bitcast_convert_type(blk_a, I32).T, I8)
        k8[2 * p + 1, cols, :] = pltpu.bitcast(lax.bitcast_convert_type(blk_b, I32).T, I8)

    def phase1(j, carry):
        r0 = pl.multiple_of(j * TS, TS)
        cols = pl.ds(r0, TS)
        xt = x_v[cols, :]
        ones8 = jnp.where(lax.broadcasted_iota(I32, (8, TS), 0) == 0, 1.0, 0.0)
        low1 = _lower(128)
        low = _lower(TS)
        sub = lax.broadcasted_iota(I32, (8, TS), 0)
        zero8 = jnp.zeros((8, TS), F32)
        proj = {}
        state = {"vm": jnp.zeros((8, TS), F32)}

        def mxu(g):
            lo, hi = GR * g, GR * (g + 1)
            proj[g] = (_dot_nt(wt1[D + lo:D + hi, :], xt), _dot_nt(wt1[2 * D + lo:2 * D + hi, :], xt),
                       _dot_nt(wt2[2 * D + 16 + lo:2 * D + 16 + hi, :], xt))

        def vpu(g):
            pk_t, vb_t, va_t = proj.pop(g)
            for i in range(GP):
                p = GP * g + i
                v = _tiles(va_t[40 * i:40 * (i + 1)])
                for a in v:
                    state["vm"] = jnp.maximum(state["vm"], jnp.abs(a))
                mid_a = jnp.where(low, v[2], jnp.where(sub == 4, 1.0, 0.0))
                mid_b = jnp.where(low, jnp.where(sub == 0, 1.0, 0.0), v[2])
                vt[2 * p, :, cols] = jnp.concatenate([v[0], v[1], mid_a, zero8], axis=0).astype(BF16)
                vt[2 * p + 1, :, cols] = jnp.concatenate([v[3], v[4], mid_b, zero8], axis=0).astype(BF16)
                phi = _feature_softmax(pk_t[40 * i:40 * (i + 1)]).astype(BF16)
                vaug = jnp.concatenate([vb_t[40 * i:40 * (i + 1)], ones8], axis=0).astype(BF16)
                kv[p, :, 0:80] = kv[p, :, 0:80] + _dot_nt(vaug, phi)
                key_digits(p, r0, cols, low1)

        for i in range(2):
            r = pl.multiple_of(jnp.minimum(2 * j + i, 4) * 128, 128)
            wt2[pl.ds(r, 128), :] = waqv_v[:, pl.ds(r, 128)].T
        mxu(0)
        for g in range(NG):
            if g + 1 < NG:
                mxu(g + 1)
            vpu(g)
        vm = state["vm"]
        for b in range(4):
            chk[8:16, :] = jnp.maximum(chk[8:16, :], vm[:, 128 * b:128 * (b + 1)])
        return carry

    lax.fori_loop(0, NTS, phase1, 0)

    kvv = kv[...]
    r = lax.broadcasted_iota(I32, (NP, 48, 128), 1)
    c = lax.broadcasted_iota(I32, (NP, 48, 128), 2)
    col_a = (c < 20) | ((c >= 40) & (c < 60))
    col_b = ((c >= 20) & (c < 40)) | ((c >= 60) & (c < 80))
    row_a = (r < 20) | (r == 40)
    row_b = ((r >= 20) & (r < 40)) | (r == 41)
    src = jnp.where(r >= 40, jnp.broadcast_to(kvv[:, 40:41, :], (NP, 48, 128)), kvv)
    lmat[...] = jnp.where((row_a & col_a) | (row_b & col_b), src, 0.0).astype(BF16)

    cp_woa.wait()
    cp_wob.wait()

    def phase2(j, carry):
        r0 = pl.multiple_of(j * TS, TS)
        cols = pl.ds(r0, TS)
        xt = x_v[cols, :]
        for i in range(3):
            r = pl.multiple_of(jnp.minimum(3 * j + i, 9) * 128, 128)
            wot[:, pl.ds(r, 128)] = wo_v[pl.ds(r, 128), :].T
        first = _dot_nt(wt2[0:D + 16, :], xt)
        g = jax.nn.sigmoid(first[D:D + 1])
        g_v[:, cols] = jnp.broadcast_to(g, (8, TS))
        low = _lower(TS)
        low1 = _lower(128)
        shift_q = jnp.full((8, 128), 127, I32)
        proj = {}
        state = {"ok": jnp.ones((1, 128), F32)}

        def mxu(gi):
            lo, hi = GR * gi, GR * (gi + 1)
            proj[gi] = (_dot_nt(wt2[D + 16 + lo:D + 16 + hi, :], xt), first[lo:hi])

        def vpu(gi):
            pq_t, q_t = proj.pop(gi)
            for i in range(GP):
                p = GP * gi + i
                phi = _feature_softmax(pq_t[40 * i:40 * (i + 1)]).astype(BF16)
                nd = _dot(lmat[p, :, 0:80], phi)
                rr = _seg_bcast((1.0 - g) * _recip(nd[40:41] + 1e-6), (1.0 - g) * _recip(nd[41:42] + 1e-6), low)
                ob = jnp.concatenate([a * b for a, b in zip(_tiles(nd[0:40]), rr)], axis=0)
                ot[D + 40 * p:D + 40 * (p + 1), cols] = ob.astype(BF16)
                kcp = kcol[40 * p:40 * (p + 1), :]
                for t in range(4):
                    tc = pl.ds(r0 + 128 * t, 128)
                    z = _tiles(q_t[40 * i:40 * (i + 1), 128 * t:128 * (t + 1)] * kcp)
                    az = [jnp.abs(a) for a in z]
                    m_a, m_b = _seg_reduce(az, jnp.maximum, jnp.max, 0.0, low1)
                    m_a = jnp.maximum(m_a, TINY)
                    m_b = jnp.maximum(m_b, TINY)
                    inv = _seg_bcast(FS * _recip(m_a), FS * _recip(m_b), low1)
                    bits = [lax.bitcast_convert_type(a * s_ + MAGIC, I32) for a, s_ in zip(z, inv)]
                    x0 = [(u << 20) >> 28 for u in bits]
                    x1 = [((u >> 4) & 15) - 8 for u in bits]
                    x2 = [(u & 15) - 8 for u in bits]
                    slots = [[a << 4 for a in x0], [a << 2 for a in x0], [a << 2 for a in x1], x1, x0, x2]
                    sig_a = m_a * (256.0 / (FS * FS))
                    sig_b = m_b * (256.0 / (FS * FS))
                    blk_a, blk_b = _head_blocks(slots, low1, shift_q, shift_q)
                    q8t[2 * p, :, tc] = blk_a.astype(I8)
                    q8t[2 * p + 1, :, tc] = blk_b.astype(I8)
                    sc[2 * p, :, tc] = jnp.broadcast_to(sig_a, (8, 128))
                    sc[2 * p + 1, :, tc] = jnp.broadcast_to(sig_b, (8, 128))
                    state["ok"] = jnp.minimum(
                        state["ok"], jnp.where(jnp.logical_and(m_a <= Q_MAX, m_b <= Q_MAX), 1.0, 0.0))

        mxu(0)
        for gi in range(NG):
            if gi + 1 < NG:
                mxu(gi + 1)
            vpu(gi)
        chk[0:1, :] = jnp.minimum(chk[0:1, :], state["ok"])
        return carry

    lax.fori_loop(0, NTS, phase2, 0)

    vmax = jnp.max(chk[8:16, :])
    fast = jnp.logical_and(jnp.min(chk[0:8, :]) > 0.5, jnp.logical_and(vmax >= V_MIN, vmax <= V_MAX))

    def finish_pair(p, acc_a, acc_b, cols, n):
        low = _lower(n)
        g = g_v[0:1, cols]
        ra = g * _recip(acc_a[20:21])
        rb = g * _recip(acc_b[16:17])
        o = jnp.concatenate([acc_a[0:8] * ra, acc_a[8:16] * ra,
                             jnp.where(low, acc_a[16:24] * ra, acc_b[16:24] * rb),
                             acc_b[0:8] * rb, acc_b[8:16] * rb], axis=0)
        ot[pl.ds(pl.multiple_of(40 * p, 8), 40), cols] = o.astype(BF16)

    @pl.when(fast)
    def _():
        nq = S // TQ
        nt = TQ // 128
        nch = S // CH

        def pair_body(pb, carry):
            steps = [(qi, u) for pp in range(PB) for qi in range(nq) for u in range(2 * pp, 2 * pp + 2)]
            pv = {}
            acc = {}

            def stage_a(g):
                s, j = divmod(g, nch)
                qi, u = steps[s]
                h = 2 * PB * pb + u
                z = jnp.dot(k8[h, j * CH:(j + 1) * CH, :], q8t[h, :, qi * TQ:(qi + 1) * TQ],
                            preferred_element_type=I32)
                for t in range(nt):
                    c0 = qi * TQ + t * 128
                    sig = sc[h, 0:1, c0:c0 + 128]
                    pv[(g, t)] = jnp.exp2(z[:, t * 128:(t + 1) * 128].astype(F32) * sig)

            nsub = CH // CB

            def stage_b(g, i):
                s, j = divmod(g, nch)
                qi, u = steps[s]
                h = 2 * PB * pb + u
                r0 = j * CH + i * CB
                v = vt[h, :, r0:r0 + CB]
                ds = [_dot(v, pv[(g, t)][i * CB:(i + 1) * CB].astype(BF16))[0:24] for t in range(nt)]
                acc[s] = ds if (j == 0 and i == 0) else [a + b for a, b in zip(acc[s], ds)]
                if j == nch - 1 and i == nsub - 1 and u % 2 == 1:
                    for t in range(nt):
                        c0 = qi * TQ + t * 128
                        finish_pair(PB * pb + u // 2, acc[s - 1][t], acc[s][t], pl.ds(c0, 128), 128)

            total = len(steps) * nch
            seq = [(g, i) for g in range(total) for i in range(nsub)]
            done = 0
            for g in range(total):
                stage_a(g)
                if (g + 1) % AG:
                    continue
                while done < (g + 1) * nsub - SK:
                    stage_b(*seq[done])
                    done += 1
            while done < len(seq):
                stage_b(*seq[done])
                done += 1
            return carry

        lax.fori_loop(0, NP // PB, pair_body, 0)

    @pl.when(jnp.logical_not(fast))
    def _():
        def proj(j, carry):
            cols = pl.ds(pl.multiple_of(j * 128, 128), 128)
            xt = x_v[cols, :]
            kt[:, cols] = _dot_nt(wt1[0:D, :], xt)
            qtf[:, cols] = _dot_nt(wt2[0:D, :], xt) * QSCALE
            return carry

        lax.fori_loop(0, S // 128, proj, 0)
        tf = 128

        def body(i, carry):
            p = i // (S // tf)
            cols = pl.ds(pl.multiple_of((i % (S // tf)) * tf, tf), tf)
            rows = pl.ds(pl.multiple_of(40 * p, 8), 40)
            kp = kt[rows, :].astype(BF16)
            qp = qtf[rows, cols]
            first = lax.broadcasted_iota(I32, (40, tf), 0) < 20
            accs = []
            for u in range(2):
                qm = jnp.where(first if u == 0 else jnp.logical_not(first), qp, 0.0).astype(BF16)
                s_t = lax.dot_general(kp, qm, TN_DIMS, preferred_element_type=F32)
                pr = jnp.exp2(s_t - jnp.max(s_t, axis=0, keepdims=True)).astype(BF16)
                accs.append(_dot(vt[2 * p + u], pr)[0:24])
            finish_pair(p, accs[0], accs[1], cols, tf)
            return carry

        lax.fori_loop(0, NP * (S // tf), body, 0)

    pieces = [(j * TS, TS) for j in range(NTS - 1)] + [(S - TS, TS // 2), (S - TS // 2, TS // 2)]
    out_copies = []
    for n, (c0, w) in enumerate(pieces):
        o_t = _dot(wot[...], ot[:, c0:c0 + w])
        ostage[c0:c0 + w, :] = o_t.T.astype(BF16)
        cp = pltpu.make_async_copy(ostage.at[c0:c0 + w, :], out_hbm.at[0, c0:c0 + w, :], out_sems.at[n])
        cp.start()
        out_copies.append(cp)
    for cp in out_copies:
        cp.wait()


def _build():
    any_spec = pl.BlockSpec(memory_space=pl.ANY)
    scratch = [
        pltpu.VMEM((S, D), BF16),
        pltpu.VMEM((S, D), BF16),
        pltpu.VMEM((D, D), BF16),
        pltpu.VMEM((D, 2 * D), BF16),
        pltpu.VMEM((D, 3 * D), BF16),
        pltpu.VMEM((2 * D, D), BF16),
        pltpu.VMEM((2 * D, D), BF16),
        pltpu.VMEM((D, 2 * D), BF16),
        pltpu.VMEM((DH, DH, H), BF16),
        pltpu.VMEM((D, 128), F32),
        pltpu.VMEM((D,), BF16),
        pltpu.VMEM((3 * D, D), BF16),
        pltpu.VMEM((3 * D + 16, D), BF16),
        pltpu.VMEM((5, TS, 128), F32),
        pltpu.VMEM((D, S), F32),
        pltpu.VMEM((D, 128), F32),
        pltpu.VMEM((D, 128), F32),
        pltpu.VMEM((NP, 48, 128), F32),
        pltpu.VMEM((NP, 48, 128), BF16),
        pltpu.VMEM((H, 128, S), I8),
        pltpu.VMEM((H, S, 128), I8),
        pltpu.VMEM((H, 32, S), BF16),
        pltpu.VMEM((H, 8, S), F32),
        pltpu.VMEM((8, S), F32),
        pltpu.VMEM((2 * D, S), BF16),
        pltpu.VMEM((S, D), BF16),
        pltpu.VMEM((16, 128), F32),
        pltpu.VMEM((D, S), F32),
        pltpu.SemaphoreType.DMA((12,)),
        pltpu.SemaphoreType.DMA((NTS + 1,)),
    ]
    return pl.pallas_call(
        _kernel,
        out_shape=jax.ShapeDtypeStruct((1, S, D), BF16),
        in_specs=[any_spec] * 7,
        out_specs=any_spec,
        scratch_shapes=scratch,
        compiler_params=pltpu.CompilerParams(vmem_limit_bytes=100 * 1024 * 1024),
        name="gated_mix_attn",
    )


@jax.jit
def pallas_gated_mix__mha_block__linear_kernel_hedgehog__prompt_kernel(
    A_x: jax.Array,
    A_wqkv: jax.Array,
    A_wo: jax.Array,
    B_x: jax.Array,
    B_wqkv: jax.Array,
    B_w_phi: jax.Array,
    B_wo: jax.Array,
    gate_w: jax.Array,
):
    del B_x
    w_phi = jnp.transpose(B_w_phi, (1, 2, 0))
    return _build()(A_x, A_wqkv, A_wo, B_wqkv, w_phi, B_wo, gate_w)
```

```python
import jax
import jax.numpy as jnp
from jax import lax
import jax.experimental.pallas as pl
import jax.experimental.pallas.tpu as pltpu

F32 = jnp.float32
BF16 = jnp.bfloat16
I32 = jnp.int32
U32 = jnp.uint32
I8 = jnp.int8

S = 2048
D = 640
H = 32
DH = 20
NP = H // 2
TS = 512
NTS = S // TS
GP = 16
GR = 40 * GP
NG = NP // GP
LOG2E = 1.4426950408889634
QSCALE = (DH ** -0.5) * LOG2E
FS = 1911.0
MAGIC = 12582912.0 + 136.0
TINY = 1e-30
Q_MAX = 3.5
V_MIN = 2.0 ** -16
V_MAX = 2.0 ** 60

NT_DIMS = (((1,), (1,)), ((), ()))
TN_DIMS = (((0,), (0,)), ((), ()))

TQ = 512
CH = 128
CB = 128
AG = 2
PB = 2
SK = 2


def _dot(a, b):
    return jnp.dot(a, b, preferred_element_type=F32)


def _dot_nt(a, b):
    return lax.dot_general(a, b, NT_DIMS, preferred_element_type=F32)


def _recip(x):
    r = pl.reciprocal(x, approx=True)
    return r * (2.0 - x * r)


def _transpose_into(dst, row0, src, col0, ncols):
    for c in range(0, ncols, 128):
        dst[row0 + c:row0 + c + 128, :] = src[:, col0 + c:col0 + c + 128].T


def _lower(n):
    return lax.broadcasted_iota(I32, (8, n), 0) < 4


def _seg_reduce(v, op, red, fill, low):
    a = op(op(v[0], v[1]), jnp.where(low, v[2], fill))
    b = op(op(v[3], v[4]), jnp.where(low, fill, v[2]))
    return red(a, axis=0, keepdims=True), red(b, axis=0, keepdims=True)


def _seg_bcast(a, b, low):
    n = a.shape[-1]
    a8 = jnp.broadcast_to(a, (8, n))
    b8 = jnp.broadcast_to(b, (8, n))
    return [a8, a8, jnp.where(low, a8, b8), b8, b8]


def _tiles(z):
    return [z[8 * i:8 * (i + 1)] for i in range(z.shape[0] // 8)]


def _feature_softmax(z):
    n = z.shape[-1]
    low = _lower(n)
    v = _tiles(z)
    mx = _seg_bcast(*_seg_reduce(v, jnp.maximum, jnp.max, -jnp.inf, low), low)
    mn = _seg_bcast(*_seg_reduce(v, jnp.minimum, jnp.min, jnp.inf, low), low)
    ep = [jnp.exp2(a - m) for a, m in zip(v, mx)]
    en = [jnp.exp2(m - a) for a, m in zip(v, mn)]
    sa, sb = _seg_reduce(ep, jnp.add, jnp.sum, 0.0, low)
    rp = _seg_bcast(_recip(sa), _recip(sb), low)
    sa, sb = _seg_reduce(en, jnp.add, jnp.sum, 0.0, low)
    rn = _seg_bcast(_recip(sa), _recip(sb), low)
    return jnp.concatenate([e * r for e, r in zip(ep, rp)] + [e * r for e, r in zip(en, rn)], axis=0)


def _head_blocks(slots, low, last_a, last_b):
    blk_a, blk_b = [], []
    for t in range(6):
        blk_a += [slots[t][0], slots[t][1]]
        blk_b += [slots[t][3], slots[t][4]]
    for t in range(0, 6, 2):
        lo, hi = slots[t][2], slots[t + 1][2]
        blk_a.append(jnp.where(low, lo, pltpu.roll(hi, 4, 0)))
        blk_b.append(jnp.where(low, pltpu.roll(lo, 4, 0), hi))
    blk_a.append(last_a)
    blk_b.append(last_b)
    return jnp.concatenate(blk_a, axis=0), jnp.concatenate(blk_b, axis=0)


def _kernel(x_hbm, wa_hbm, woa_hbm, wb_hbm, wphi_hbm, wob_hbm, gate_hbm, out_hbm,
            x_v, xp_v, wak_v, waqv_v, wb_v, wbt, wo_v, wot, wphi_v, w2s, gate_v, wt1, wt2, xs, kt, kcol, kinv_v, kv, lmat,
            q8t, k8, vt, sc, g_v, ot, ostage, chk, qtf, in_sems, out_sems):
    cp_x = [pltpu.make_async_copy(x_hbm.at[0, pl.ds(j * TS, TS), :], x_v.at[pl.ds(j * TS, TS), :], in_sems.at[j])
            for j in range(NTS)]
    cp_wk = pltpu.make_async_copy(wa_hbm.at[:, pl.ds(D, D)], wak_v, in_sems.at[4])
    cp_wb = pltpu.make_async_copy(wb_hbm, wb_v, in_sems.at[5])
    cp_phi = pltpu.make_async_copy(wphi_hbm, wphi_v, in_sems.at[6])
    cp_gate = pltpu.make_async_copy(gate_hbm, gate_v, in_sems.at[7])
    cp_wq = pltpu.make_async_copy(wa_hbm.at[:, pl.ds(0, D)], waqv_v.at[:, pl.ds(0, D)], in_sems.at[8])
    cp_wv = pltpu.make_async_copy(wa_hbm.at[:, pl.ds(2 * D, D)], waqv_v.at[:, pl.ds(D, D)], in_sems.at[9])
    cp_woa = pltpu.make_async_copy(woa_hbm, wo_v.at[0:D], in_sems.at[10])
    cp_wob = pltpu.make_async_copy(wob_hbm, wo_v.at[D:2 * D], in_sems.at[11])
    for c in (cp_x[0], cp_x[1], cp_wk, cp_x[2], cp_x[3], cp_wb, cp_phi, cp_gate):
        c.start()
    chk[...] = jnp.concatenate([jnp.ones((8, 128), F32), jnp.zeros((8, 128), F32)], axis=0)

    def permute(j):
        r0 = j * TS
        for c in range(5):
            xs[c] = x_v[r0:r0 + TS, 128 * c:128 * (c + 1)].astype(F32)
        for b in range(4):
            xp_v[r0 + 128 * b:r0 + 128 * (b + 1), :] = jnp.concatenate(
                [xs[c, pl.ds(b, 128, stride=4), :] for c in range(5)], axis=1).astype(BF16)

    def keys(j):
        r0 = j * TS
        k_t = _dot_nt(wt1[0:D, :], xp_v[r0:r0 + TS, :])
        kt[:, r0:r0 + TS] = k_t
        ak = jnp.abs(k_t)
        m = ak[:, 0:128]
        fin = ak[:, 0:128] < jnp.inf
        for b in range(1, 4):
            m = jnp.maximum(m, ak[:, 128 * b:128 * (b + 1)])
            fin = jnp.logical_and(fin, ak[:, 128 * b:128 * (b + 1)] < jnp.inf)
        kcol[...] = m if j == 0 else jnp.maximum(kcol[...], m)
        okf = jnp.min(jnp.where(fin, 1.0, 0.0).reshape(D // 8, 8, 128), axis=0)
        chk[0:8, :] = jnp.minimum(chk[0:8, :], okf)

    cp_x[0].wait()
    permute(0)
    cp_x[1].wait()
    permute(1)
    cp_wk.wait()
    _transpose_into(wt1, 0, wak_v, 0, D)
    keys(0)
    cp_x[2].wait()
    cp_x[3].wait()
    cp_wv.start()
    cp_wq.start()
    permute(2)
    keys(1)
    permute(3)
    keys(2)
    cp_wb.wait()
    cp_phi.wait()
    cp_gate.wait()
    cp_wv.wait()
    _transpose_into(wbt, D, wb_v, D, D)
    keys(3)
    kv[...] = jnp.zeros_like(kv)
    for blk in range(5):
        rows = []
        for dl in range(4):
            a = wphi_v[4 * blk + dl].astype(F32)
            rows += [jnp.concatenate([a, jnp.zeros((DH, 128 - H), F32)], axis=1), jnp.zeros((12, 128), F32)]
        t = jnp.concatenate(rows, axis=0).T[0:H]
        for dl in range(4):
            w2s[pl.ds(4 * blk + dl, H, stride=DH), :] = t if dl == 0 else pltpu.roll(t, 128 - 32 * dl, 1)
    row = lax.broadcasted_iota(I32, (40, 128), 0)
    lane = lax.broadcasted_iota(I32, (40, 128), 1)
    lhs = []
    for p in range(NP):
        a = w2s[40 * p:40 * (p + 1), :]
        m = jnp.where(row < DH, jnp.where(lane < DH, a, 0.0),
                      jnp.where((lane >= DH) & (lane < 2 * DH), pltpu.roll(a, DH, 1), 0.0))
        lhs.append(m.T[0:48].astype(BF16))
    for p in range(NP):
        res = _dot(lhs[p], wbt[D + 40 * p:D + 40 * (p + 1), :])
        wt1[D + 40 * p:D + 40 * (p + 1), :] = (res[0:40] * LOG2E).astype(BF16)
    _transpose_into(wt1, 2 * D, wb_v, 2 * D, D)
    _transpose_into(wt2, 2 * D + 16, waqv_v, D, D)
    _transpose_into(wbt, 0, wb_v, 0, D)
    for p in range(NP):
        res = _dot(lhs[p], wbt[40 * p:40 * (p + 1), :])
        wt2[D + 16 + 40 * p:D + 16 + 40 * (p + 1), :] = (res[0:40] * LOG2E).astype(BF16)
    grow = jnp.broadcast_to(gate_v[...].astype(F32).reshape(1, D), (16, D))
    wt2[D:D + 16, :] = grow.astype(BF16)
    kc = jnp.maximum(jnp.max(kcol[...], axis=1, keepdims=True), TINY)
    kinv_v[...] = jnp.broadcast_to(FS / kc, (D, 128))
    kcol[...] = jnp.broadcast_to(kc * QSCALE, (D, 128))
    cp_woa.start()
    cp_wob.start()
    cp_wq.wait()

    def key_digits(p, r0, cols, low1):
        kinv = kinv_v[40 * p:40 * (p + 1), :]
        w0 = w1 = w2_ = None
        for b in range(4):
            y = kt[40 * p:40 * (p + 1), pl.ds(r0 + 128 * b, 128)] * kinv + MAGIC
            u = lax.bitcast_convert_type(y, U32)
            msk = jnp.uint32(15 << (8 * b))
            n2 = (u << (8 * b)) & msk
            n1 = ((u >> 4) if b == 0 else (u << (8 * b - 4))) & msk
            n0 = ((u >> 8) if b == 0 else (u if b == 1 else (u << (8 * b - 8)))) & msk
            w0 = n0 if b == 0 else w0 | n0
            w1 = n1 if b == 0 else w1 | n1
            w2_ = n2 if b == 0 else w2_ | n2
        c78 = jnp.uint32(0x78787878)
        c80 = jnp.uint32(0x80808080)
        w0 = ((w0 ^ jnp.uint32(0x08080808)) + c78) ^ c80
        w1 = (w1 + c78) ^ c80
        w2_ = (w2_ + c78) ^ c80
        cf0 = jnp.uint32(0xF0F0F0F0)
        cfc = jnp.uint32(0xFCFCFCFC)
        slots = [_tiles((w0 << 4) & cf0), _tiles((w1 << 2) & cfc), _tiles((w0 << 2) & cfc),
                 _tiles(w1), _tiles(w2_), _tiles(w0)]
        shift_w = jnp.where(lax.broadcasted_iota(I32, (8, 128), 0) == 0,
                            jnp.uint32(0xFFFFFFFF), jnp.uint32(0x80808080))
        blk_a, blk_b = _head_blocks(slots, low1, shift_w, shift_w)
        k8[2 * p, cols, :] = pltpu.bitcast(lax.bitcast_convert_type(blk_a, I32).T, I8)
        k8[2 * p + 1, cols, :] = pltpu.bitcast(lax.bitcast_convert_type(blk_b, I32).T, I8)

    def phase1(j, carry):
        r0 = pl.multiple_of(j * TS, TS)
        cols = pl.ds(r0, TS)
        xt = x_v[cols, :]
        ones8 = jnp.where(lax.broadcasted_iota(I32, (8, TS), 0) == 0, 1.0, 0.0)
        low1 = _lower(128)
        low = _lower(TS)
        sub = lax.broadcasted_iota(I32, (8, TS), 0)
        zero8 = jnp.zeros((8, TS), F32)
        proj = {}
        state = {"vm": jnp.zeros((8, TS), F32)}

        def mxu(g):
            lo, hi = GR * g, GR * (g + 1)
            proj[g] = (_dot_nt(wt1[D + lo:D + hi, :], xt), _dot_nt(wt1[2 * D + lo:2 * D + hi, :], xt),
                       _dot_nt(wt2[2 * D + 16 + lo:2 * D + 16 + hi, :], xt))

        def vpu(g):
            pk_t, vb_t, va_t = proj.pop(g)
            for i in range(GP):
                p = GP * g + i
                v = _tiles(va_t[40 * i:40 * (i + 1)])
                for a in v:
                    state["vm"] = jnp.maximum(state["vm"], jnp.abs(a))
                mid_a = jnp.where(low, v[2], jnp.where(sub == 4, 1.0, 0.0))
                mid_b = jnp.where(low, jnp.where(sub == 0, 1.0, 0.0), v[2])
                vt[2 * p, :, cols] = jnp.concatenate([v[0], v[1], mid_a, zero8], axis=0).astype(BF16)
                vt[2 * p + 1, :, cols] = jnp.concatenate([v[3], v[4], mid_b, zero8], axis=0).astype(BF16)
                phi = _feature_softmax(pk_t[40 * i:40 * (i + 1)]).astype(BF16)
                vaug = jnp.concatenate([vb_t[40 * i:40 * (i + 1)], ones8], axis=0).astype(BF16)
                kv[p, :, 0:80] = kv[p, :, 0:80] + _dot_nt(vaug, phi)
                key_digits(p, r0, cols, low1)

        for i in range(2):
            r = pl.multiple_of(jnp.minimum(2 * j + i, 4) * 128, 128)
            wt2[pl.ds(r, 128), :] = waqv_v[:, pl.ds(r, 128)].T
        mxu(0)
        for g in range(NG):
            if g + 1 < NG:
                mxu(g + 1)
            vpu(g)
        vm = state["vm"]
        for b in range(4):
            chk[8:16, :] = jnp.maximum(chk[8:16, :], vm[:, 128 * b:128 * (b + 1)])
        return carry

    lax.fori_loop(0, NTS, phase1, 0)

    kvv = kv[...]
    r = lax.broadcasted_iota(I32, (NP, 48, 128), 1)
    c = lax.broadcasted_iota(I32, (NP, 48, 128), 2)
    col_a = (c < 20) | ((c >= 40) & (c < 60))
    col_b = ((c >= 20) & (c < 40)) | ((c >= 60) & (c < 80))
    row_a = (r < 20) | (r == 40)
    row_b = ((r >= 20) & (r < 40)) | (r == 41)
    src = jnp.where(r >= 40, jnp.broadcast_to(kvv[:, 40:41, :], (NP, 48, 128)), kvv)
    lmat[...] = jnp.where((row_a & col_a) | (row_b & col_b), src, 0.0).astype(BF16)

    cp_woa.wait()
    cp_wob.wait()

    def phase2(j, carry):
        r0 = pl.multiple_of(j * TS, TS)
        cols = pl.ds(r0, TS)
        xt = x_v[cols, :]
        for i in range(3):
            r = pl.multiple_of(jnp.minimum(3 * j + i, 9) * 128, 128)
            wot[:, pl.ds(r, 128)] = wo_v[pl.ds(r, 128), :].T
        first = _dot_nt(wt2[0:D + 16, :], xt)
        g = jax.nn.sigmoid(first[D:D + 1])
        g_v[:, cols] = jnp.broadcast_to(g, (8, TS))
        low = _lower(TS)
        low1 = _lower(128)
        shift_q = jnp.full((8, 128), 127, I32)
        proj = {}
        state = {"ok": jnp.ones((1, 128), F32)}

        def mxu(gi):
            lo, hi = GR * gi, GR * (gi + 1)
            proj[gi] = (_dot_nt(wt2[D + 16 + lo:D + 16 + hi, :], xt), first[lo:hi])

        def vpu(gi):
            pq_t, q_t = proj.pop(gi)
            for i in range(GP):
                p = GP * gi + i
                phi = _feature_softmax(pq_t[40 * i:40 * (i + 1)]).astype(BF16)
                nd = _dot(lmat[p, :, 0:80], phi)
                rr = _seg_bcast((1.0 - g) * _recip(nd[40:41] + 1e-6), (1.0 - g) * _recip(nd[41:42] + 1e-6), low)
                ob = jnp.concatenate([a * b for a, b in zip(_tiles(nd[0:40]), rr)], axis=0)
                ot[D + 40 * p:D + 40 * (p + 1), cols] = ob.astype(BF16)
                kcp = kcol[40 * p:40 * (p + 1), :]
                for t in range(4):
                    tc = pl.ds(r0 + 128 * t, 128)
                    z = _tiles(q_t[40 * i:40 * (i + 1), 128 * t:128 * (t + 1)] * kcp)
                    az = [jnp.abs(a) for a in z]
                    m_a, m_b = _seg_reduce(az, jnp.maximum, jnp.max, 0.0, low1)
                    m_a = jnp.maximum(m_a, TINY)
                    m_b = jnp.maximum(m_b, TINY)
                    inv = _seg_bcast(FS * _recip(m_a), FS * _recip(m_b), low1)
                    bits = [lax.bitcast_convert_type(a * s_ + MAGIC, I32) for a, s_ in zip(z, inv)]
                    x0 = [(u << 20) >> 28 for u in bits]
                    x1 = [((u >> 4) & 15) - 8 for u in bits]
                    x2 = [(u & 15) - 8 for u in bits]
                    slots = [[a << 4 for a in x0], [a << 2 for a in x0], [a << 2 for a in x1], x1, x0, x2]
                    sig_a = m_a * (256.0 / (FS * FS))
                    sig_b = m_b * (256.0 / (FS * FS))
                    blk_a, blk_b = _head_blocks(slots, low1, shift_q, shift_q)
                    q8t[2 * p, :, tc] = blk_a.astype(I8)
                    q8t[2 * p + 1, :, tc] = blk_b.astype(I8)
                    sc[2 * p, :, tc] = jnp.broadcast_to(sig_a, (8, 128))
                    sc[2 * p + 1, :, tc] = jnp.broadcast_to(sig_b, (8, 128))
                    state["ok"] = jnp.minimum(
                        state["ok"], jnp.where(jnp.logical_and(m_a <= Q_MAX, m_b <= Q_MAX), 1.0, 0.0))

        mxu(0)
        for gi in range(NG):
            if gi + 1 < NG:
                mxu(gi + 1)
            vpu(gi)
        chk[0:1, :] = jnp.minimum(chk[0:1, :], state["ok"])
        return carry

    lax.fori_loop(0, NTS, phase2, 0)

    vmax = jnp.max(chk[8:16, :])
    fast = jnp.logical_and(jnp.min(chk[0:8, :]) > 0.5, jnp.logical_and(vmax >= V_MIN, vmax <= V_MAX))

    def finish_pair(p, acc_a, acc_b, cols, n):
        low = _lower(n)
        g = g_v[0:1, cols]
        ra = g * _recip(acc_a[20:21])
        rb = g * _recip(acc_b[16:17])
        o = jnp.concatenate([acc_a[0:8] * ra, acc_a[8:16] * ra,
                             jnp.where(low, acc_a[16:24] * ra, acc_b[16:24] * rb),
                             acc_b[0:8] * rb, acc_b[8:16] * rb], axis=0)
        ot[pl.ds(pl.multiple_of(40 * p, 8), 40), cols] = o.astype(BF16)

    @pl.when(fast)
    def _():
        nq = S // TQ
        nt = TQ // 128
        nch = S // CH

        def pair_body(pb, carry):
            steps = [(qi, u) for pp in range(PB) for qi in range(nq) for u in range(2 * pp, 2 * pp + 2)]
            pv = {}
            acc = {}

            def stage_a(g):
                s, j = divmod(g, nch)
                qi, u = steps[s]
                h = 2 * PB * pb + u
                z = jnp.dot(k8[h, j * CH:(j + 1) * CH, :], q8t[h, :, qi * TQ:(qi + 1) * TQ],
                            preferred_element_type=I32)
                for t in range(nt):
                    c0 = qi * TQ + t * 128
                    sig = sc[h, 0:1, c0:c0 + 128]
                    pv[(g, t)] = jnp.exp2(z[:, t * 128:(t + 1) * 128].astype(F32) * sig)

            nsub = CH // CB

            def stage_b(g, i):
                s, j = divmod(g, nch)
                qi, u = steps[s]
                h = 2 * PB * pb + u
                r0 = j * CH + i * CB
                v = vt[h, :, r0:r0 + CB]
                ds = [_dot(v, pv[(g, t)][i * CB:(i + 1) * CB].astype(BF16))[0:24] for t in range(nt)]
                acc[s] = ds if (j == 0 and i == 0) else [a + b for a, b in zip(acc[s], ds)]
                if j == nch - 1 and i == nsub - 1 and u % 2 == 1:
                    for t in range(nt):
                        c0 = qi * TQ + t * 128
                        finish_pair(PB * pb + u // 2, acc[s - 1][t], acc[s][t], pl.ds(c0, 128), 128)

            total = len(steps) * nch
            seq = [(g, i) for g in range(total) for i in range(nsub)]
            done = 0
            for g in range(total):
                stage_a(g)
                if (g + 1) % AG:
                    continue
                while done < (g + 1) * nsub - SK:
                    stage_b(*seq[done])
                    done += 1
            while done < len(seq):
                stage_b(*seq[done])
                done += 1
            return carry

        lax.fori_loop(0, NP // PB, pair_body, 0)

    @pl.when(jnp.logical_not(fast))
    def _():
        def proj(j, carry):
            cols = pl.ds(pl.multiple_of(j * 128, 128), 128)
            xt = x_v[cols, :]
            kt[:, cols] = _dot_nt(wt1[0:D, :], xt)
            qtf[:, cols] = _dot_nt(wt2[0:D, :], xt) * QSCALE
            return carry

        lax.fori_loop(0, S // 128, proj, 0)
        tf = 128

        def body(i, carry):
            p = i // (S // tf)
            cols = pl.ds(pl.multiple_of((i % (S // tf)) * tf, tf), tf)
            rows = pl.ds(pl.multiple_of(40 * p, 8), 40)
            kp = kt[rows, :].astype(BF16)
            qp = qtf[rows, cols]
            first = lax.broadcasted_iota(I32, (40, tf), 0) < 20
            accs = []
            for u in range(2):
                qm = jnp.where(first if u == 0 else jnp.logical_not(first), qp, 0.0).astype(BF16)
                s_t = lax.dot_general(kp, qm, TN_DIMS, preferred_element_type=F32)
                pr = jnp.exp2(s_t - jnp.max(s_t, axis=0, keepdims=True)).astype(BF16)
                accs.append(_dot(vt[2 * p + u], pr)[0:24])
            finish_pair(p, accs[0], accs[1], cols, tf)
            return carry

        lax.fori_loop(0, NP * (S // tf), body, 0)

    pieces = [(0, 1024), (1024, 512), (1536, 256), (1792, 128), (1920, 128)]
    out_copies = []
    for n, (c0, w) in enumerate(pieces):
        o_t = _dot(wot[...], ot[:, c0:c0 + w])
        ostage[c0:c0 + w, :] = o_t.T.astype(BF16)
        cp = pltpu.make_async_copy(ostage.at[c0:c0 + w, :], out_hbm.at[0, c0:c0 + w, :], out_sems.at[n])
        cp.start()
        out_copies.append(cp)
    for cp in out_copies:
        cp.wait()


def _build():
    any_spec = pl.BlockSpec(memory_space=pl.ANY)
    scratch = [
        pltpu.VMEM((S, D), BF16),
        pltpu.VMEM((S, D), BF16),
        pltpu.VMEM((D, D), BF16),
        pltpu.VMEM((D, 2 * D), BF16),
        pltpu.VMEM((D, 3 * D), BF16),
        pltpu.VMEM((2 * D, D), BF16),
        pltpu.VMEM((2 * D, D), BF16),
        pltpu.VMEM((D, 2 * D), BF16),
        pltpu.VMEM((DH, DH, H), BF16),
        pltpu.VMEM((D, 128), F32),
        pltpu.VMEM((D,), BF16),
        pltpu.VMEM((3 * D, D), BF16),
        pltpu.VMEM((3 * D + 16, D), BF16),
        pltpu.VMEM((5, TS, 128), F32),
        pltpu.VMEM((D, S), F32),
        pltpu.VMEM((D, 128), F32),
        pltpu.VMEM((D, 128), F32),
        pltpu.VMEM((NP, 48, 128), F32),
        pltpu.VMEM((NP, 48, 128), BF16),
        pltpu.VMEM((H, 128, S), I8),
        pltpu.VMEM((H, S, 128), I8),
        pltpu.VMEM((H, 32, S), BF16),
        pltpu.VMEM((H, 8, S), F32),
        pltpu.VMEM((8, S), F32),
        pltpu.VMEM((2 * D, S), BF16),
        pltpu.VMEM((S, D), BF16),
        pltpu.VMEM((16, 128), F32),
        pltpu.VMEM((D, S), F32),
        pltpu.SemaphoreType.DMA((12,)),
        pltpu.SemaphoreType.DMA((5,)),
    ]
    return pl.pallas_call(
        _kernel,
        out_shape=jax.ShapeDtypeStruct((1, S, D), BF16),
        in_specs=[any_spec] * 7,
        out_specs=any_spec,
        scratch_shapes=scratch,
        compiler_params=pltpu.CompilerParams(vmem_limit_bytes=100 * 1024 * 1024),
        name="gated_mix_attn",
    )


@jax.jit
def pallas_gated_mix__mha_block__linear_kernel_hedgehog__prompt_kernel(
    A_x: jax.Array,
    A_wqkv: jax.Array,
    A_wo: jax.Array,
    B_x: jax.Array,
    B_wqkv: jax.Array,
    B_w_phi: jax.Array,
    B_wo: jax.Array,
    gate_w: jax.Array,
):
    del B_x
    w_phi = jnp.transpose(B_w_phi, (1, 2, 0))
    return _build()(A_x, A_wqkv, A_wo, B_wqkv, w_phi, B_wo, gate_w)
```
